```python
import jax
import jax.numpy as jnp

def _softmax(x, axis=-1):
    return jax.nn.softmax(x, axis=axis)

def _gelu(x):
    return jax.nn.gelu(x, approximate=True)

def _silu(x):
    return jax.nn.silu(x)

def _sigmoid(x):
    return jax.nn.sigmoid(x)

def _layernorm(x, axis=-1, eps=1e-05):
    m = jnp.mean(x, axis=axis, keepdims=True)
    v = jnp.var(x, axis=axis, keepdims=True)
    return (x - m) / jnp.sqrt(v + eps)

def _scatter_add(tgt, idx, src, axis=0):
    return tgt.at[idx].add(src)

def _segment_sum(src, seg, n):
    return jax.ops.segment_sum(src, seg, n)

class _Rng:

    def __init__(self, key):
        self._k = key

    def _next(self):
        self._k, sub = jax.random.split(self._k)
        return sub

    def normal(self, shape):
        return jax.random.normal(self._next(), shape, dtype=jnp.bfloat16)

    def randint(self, lo, hi, shape):
        return jax.random.randint(self._next(), shape, lo, hi, dtype=jnp.int32)

    def uniform(self, shape, lo=0.0, hi=1.0):
        return jax.random.uniform(self._next(), shape, jnp.bfloat16, lo, hi)

    def permutation(self, n):
        return jax.random.permutation(self._next(), n)
kernel_name = 'concat_heads__memory_aug_recurrent_mem_tr__compressed_kv_cla__prompt'

def setup_inputs():
    _rng = _Rng(jax.random.key(int.from_bytes(__import__("os").urandom(4), "little")))
    _w = lambda a: (lambda t: t.astype(jnp.bfloat16) if jnp.issubdtype(t.dtype, jnp.floating) else t)(jnp.asarray(a))

    def _A_setup():
        B, S, Dm = (1, 2048, 448)
        H, Dh = (16, 256)
        M, seg = (8, 32)
        seg = min(seg, S)
        S = S // seg * seg
        return {'x': _w((lambda *s: _rng.normal(s) * 0.05)(B, S, Dm)), 'mem0': _w((lambda *s: _rng.normal(s) * 0.05)(B, M, Dm)), 'Wq': _w((lambda *s: _rng.normal(s) * 0.05)(Dm, H, Dh) * Dm ** (-0.5)), 'Wk': _w((lambda *s: _rng.normal(s) * 0.05)(Dm, H, Dh) * Dm ** (-0.5)), 'Wv': _w((lambda *s: _rng.normal(s) * 0.05)(Dm, H, Dh) * Dm ** (-0.5)), 'Wo': _w((lambda *s: _rng.normal(s) * 0.05)(H, Dh, Dm) * (H * Dh) ** (-0.5)), 'seg_len': seg}
    _A_in = _A_setup()

    def _B_setup():
        B, H, Sq, Sk, D, M = (1, 16, 2048, 2048, 256, 448)
        Dc = 4 * D
        return {'x': _w((lambda *s: _rng.normal(s) * 0.05)(B, Sq, M)), 'c_kv': _w((lambda *s: _rng.normal(s) * 0.05)(B, Sk, Dc)), 'w_q': _w((lambda *s: _rng.normal(s) * 0.05)(M, H, D) * M ** (-0.5)), 'w_uk': _w((lambda *s: _rng.normal(s) * 0.05)(Dc, H, D) * Dc ** (-0.5)), 'w_uv': _w((lambda *s: _rng.normal(s) * 0.05)(Dc, H, D) * Dc ** (-0.5)), 'w_o': _w((lambda *s: _rng.normal(s) * 0.05)(H, D, M) * (H * D) ** (-0.5))}
    _B_in = _B_setup()
    return {'A_x': _A_in['x'], 'A_mem0': _A_in['mem0'], 'A_Wq': _A_in['Wq'], 'A_Wk': _A_in['Wk'], 'A_Wv': _A_in['Wv'], 'A_Wo': _A_in['Wo'], 'A_seg_len': _A_in['seg_len'], 'B_x': _B_in['x'], 'B_c_kv': _B_in['c_kv'], 'B_w_q': _B_in['w_q'], 'B_w_uk': _B_in['w_uk'], 'B_w_uv': _B_in['w_uv'], 'B_w_o': _B_in['w_o']}

def reference(A_x, A_mem0, A_Wq, A_Wk, A_Wv, A_Wo, A_seg_len, B_x, B_c_kv, B_w_q, B_w_uk, B_w_uv, B_w_o):

    def _A_ref(x, mem0, Wq, Wk, Wv, Wo, seg_len):
        B, S, Dm = x.shape
        H, Dh = (Wq.shape[1], Wq.shape[2])
        M = mem0.shape[1]
        scale = Dh ** (-0.5)
        n_seg = S // seg_len
        L = M + seg_len
        idx = jnp.arange(L)
        mask = (idx[:, None] < M) | (idx[:, None] >= idx[None, :])
        mem = mem0
        outs = []
        for s in range(n_seg):
            xs = x[:, s * seg_len:(s + 1) * seg_len, :].copy()
            h = jnp.concatenate([mem, xs], axis=1)
            q = jnp.einsum('btd,dhe->bhte', h, Wq)
            k = jnp.einsum('btd,dhe->bhte', h, Wk)
            v = jnp.einsum('btd,dhe->bhte', h, Wv)
            scores = jnp.einsum('bhqe,bhke->bhqk', q, k) * scale
            scores = jnp.where(mask[None, None], scores, -1000000000.0)
            p = _softmax(scores, axis=-1)
            o = jnp.einsum('bhqk,bhke->bhqe', p, v)
            o = jnp.einsum('bhte,hed->btd', o, Wo)
            mem = o[:, :M, :].copy()
            outs.append(o[:, M:, :])
        return jnp.concatenate(outs, axis=1)

    def _B_ref(x, c_kv, w_q, w_uk, w_uv, w_o):
        B, Sq, M = (x.shape[0], x.shape[1], x.shape[2])
        Sk = c_kv.shape[1]
        H, D = (w_q.shape[1], w_q.shape[2])
        q = jnp.einsum('bqm,mhd->bhqd', x, w_q)
        k = jnp.einsum('bkc,chd->bhkd', c_kv, w_uk)
        v = jnp.einsum('bkc,chd->bhkd', c_kv, w_uv)
        scores = jnp.einsum('bhqd,bhkd->bhqk', q, k) * D ** (-0.5)
        off = Sk - Sq
        qi = jnp.arange(Sq)[:, None]
        kj = jnp.arange(Sk)[None, :]
        cmask = kj <= qi + off
        scores = jnp.where(cmask[None, None], scores, -1000000000.0)
        p = _softmax(scores, axis=-1)
        ctx = jnp.einsum('bhqk,bhkd->bhqd', p, v)
        return jnp.einsum('bhqd,hdm->bqm', ctx, w_o)
    a = _A_ref(A_x, A_mem0, A_Wq, A_Wk, A_Wv, A_Wo, A_seg_len)
    b = _B_ref(B_x, B_c_kv, B_w_q, B_w_uk, B_w_uv, B_w_o)
    return jnp.concatenate([a, b], axis=-1)
```

```python
import functools

import jax
import jax.numpy as jnp
from jax import lax
import jax.experimental.pallas as pl
import jax.experimental.pallas.tpu as pltpu

S = 2048
DM = 448
H = 16
DH = 256
DC = 1024
MEM = 8
TQ = 256
CH = 64
NEG = -1000000000.0

_NN = (((1,), (0,)), ((), ()))
_NT = (((1,), (1,)), ((), ()))


def _dot(a, b, dims=_NN):
    return lax.dot_general(a, b, dims, preferred_element_type=jnp.float32)


def _deinterleave(raw, n_rows, store):
    def body(t, _):
        r0 = pl.multiple_of(t * (CH // 2), CH // 2)
        for half in range(2):
            src = raw.at[half, pl.ds(pl.multiple_of(t * (CH * 8), CH * 8), CH * 8), :]
            for j in range(8):
                x = src[pl.ds(j, CH, stride=8), :]
                lo = pltpu.bitcast(x << 16, jnp.float32).astype(jnp.bfloat16)
                hi = pltpu.bitcast(x & jnp.uint32(0xFFFF0000), jnp.float32).astype(jnp.bfloat16)
                store(2 * j, half, r0, pltpu.bitcast(lo, jnp.uint32))
                store(2 * j + 1, half, r0, pltpu.bitcast(hi, jnp.uint32))
        return 0
    lax.fori_loop(0, n_rows // CH, body, 0)


def _kernel(xa_hbm, mem_hbm, aq_hbm, ak_hbm, av_hbm, ao_hbm,
            xb_hbm, c_hbm, bq_hbm, bk_hbm, bv_hbm, bo_hbm,
            o_hbm,
            xt, xs, mem0, wao, c, wbo, raw0, raw1, raw2,
            wa, wbq, wbkv, qc, kv, out, sems, *, seg):
    def raw_copies(hbm, raw, n_rows, s0):
        u = hbm.bitcast(jnp.uint32)
        return [pltpu.make_async_copy(u.at[:, pl.ds(128 * i, 128)],
                                      raw.at[i, pl.ds(0, n_rows * 8), :],
                                      sems.at[s0 + i]) for i in range(2)]

    cp_xb = pltpu.make_async_copy(xb_hbm, xt, sems.at[0])
    cp_bq = raw_copies(bq_hbm, raw2, DM, 1)
    cp_c = pltpu.make_async_copy(c_hbm, c, sems.at[3])
    cp_bk = raw_copies(bk_hbm, raw0, DC, 4)
    cp_bv = raw_copies(bv_hbm, raw1, DC, 6)
    cp_bo = pltpu.make_async_copy(bo_hbm, wbo, sems.at[8])
    cp_xa = pltpu.make_async_copy(xa_hbm, xt, sems.at[9])
    cp_mem = pltpu.make_async_copy(mem_hbm, mem0, sems.at[10])
    cp_ao = pltpu.make_async_copy(ao_hbm, wao, sems.at[11])
    cp_aq = raw_copies(aq_hbm, raw0, DM, 12)
    cp_ak = raw_copies(ak_hbm, raw1, DM, 14)
    cp_av = raw_copies(av_hbm, raw2, DM, 16)

    cp_xb.start()
    for cp in cp_bq:
        cp.start()
    for cp in cp_bq:
        cp.wait()
    cp_c.start()
    for cp in cp_bk + cp_bv:
        cp.start()

    def st_bq(h, half, r0, val):
        wbq[h, pl.ds(r0, CH // 2), pl.ds(128 * half, 128)] = val
    _deinterleave(raw2, DM, st_bq)
    for cp in cp_av:
        cp.start()
    cp_xb.wait()

    def transpose_x():
        for m in range(S // 512):
            xs[pl.ds(m * 256, 256), :] = pltpu.bitcast(xt[:, pl.ds(m * 512, 512)].T, jnp.uint32)
    transpose_x()

    def q_body(h, _):
        w = pltpu.bitcast(wbq[h], jnp.bfloat16)
        for m in range(S // 512):
            xm = pltpu.bitcast(xs[pl.ds(m * 256, 256), :], jnp.bfloat16)
            q = _dot(xm, w) * (DH ** -0.5)
            qc[h, pl.ds(m * 256, 256), :] = pltpu.bitcast(q.astype(jnp.bfloat16), jnp.uint32)
        return 0
    lax.fori_loop(0, H, q_body, 0)

    for cp in cp_bk + cp_bv:
        cp.wait()
    cp_bo.start()
    cp_xa.start()
    cp_mem.start()
    cp_ao.start()

    def st_bk(h, half, r0, val):
        wbkv[h, pl.ds(r0, CH // 2), pl.ds(128 * half, 128)] = val

    def st_bv(h, half, r0, val):
        wbkv[h, pl.ds(r0, CH // 2), pl.ds(DH + 128 * half, 128)] = val
    _deinterleave(raw0, DC, st_bk)
    _deinterleave(raw1, DC, st_bv)
    for cp in cp_aq + cp_ak:
        cp.start()
    cp_c.wait()

    def head_body(h, _):
        w = pltpu.bitcast(wbkv[h], jnp.bfloat16)
        for m in range(S // 256):
            r = _dot(c[pl.ds(m * 256, 256), :], w)
            kv[pl.ds(m * 128, 128), :] = pltpu.bitcast(r.astype(jnp.bfloat16), jnp.uint32)
        row = lax.broadcasted_iota(jnp.int32, (TQ, TQ), 0)
        col = lax.broadcasted_iota(jnp.int32, (TQ, TQ), 1)
        for i in range(S // TQ):
            n = (i + 1) * TQ
            qrows = pl.ds(i * TQ // 2, TQ // 2)
            q = pltpu.bitcast(qc[h, qrows, :], jnp.bfloat16)
            k = pltpu.bitcast(kv[pl.ds(0, n // 2), pl.ds(0, DH)], jnp.bfloat16)
            s = _dot(q, k, _NT)
            sd = jnp.where(col <= row, s[:, n - TQ:], NEG)
            s = sd if i == 0 else jnp.concatenate([s[:, :n - TQ], sd], axis=1)
            m = jnp.max(s, axis=1, keepdims=True)
            p = jnp.exp(s - m)
            l = jnp.sum(p, axis=1, keepdims=True)
            v = pltpu.bitcast(kv[pl.ds(0, n // 2), pl.ds(DH, DH)], jnp.bfloat16)
            o = _dot(p.astype(jnp.bfloat16), v) / l
            qc[h, qrows, :] = pltpu.bitcast(o.astype(jnp.bfloat16), jnp.uint32)
        return 0
    lax.fori_loop(0, H, head_body, 0)

    for cp in cp_aq + cp_ak + cp_av:
        cp.wait()
    for t, raw in enumerate((raw0, raw1, raw2)):
        def st_a(h, half, r0, val, t=t):
            wa[h, pl.ds(r0, CH // 2), pl.ds(t * DH + 128 * half, 128)] = val
        _deinterleave(raw, DM, st_a)
    cp_xa.wait()
    transpose_x()
    cp_mem.wait()
    cp_ao.wait()
    cp_bo.wait()

    L = MEM + seg

    def a_body(sidx, mem):
        r0 = pl.multiple_of(sidx * seg, seg)
        xseg = pltpu.bitcast(xs[pl.ds(pl.multiple_of(sidx * (seg // 2), seg // 2), seg // 2), :], jnp.bfloat16)
        hx = jnp.concatenate([mem, xseg.astype(jnp.float32)], axis=0)
        row = lax.broadcasted_iota(jnp.int32, (L, L), 0)
        col = lax.broadcasted_iota(jnp.int32, (L, L), 1)
        mask = (row < MEM) | (row >= col)
        qs, ks, vs, ss, ps, os_ = {}, {}, {}, {}, {}, {}
        acc = None
        for t in range(H + 4):
            if t < H:
                qkv = _dot(hx, pltpu.bitcast(wa[t], jnp.bfloat16))
                qs[t] = qkv[:, :DH]
                ks[t] = qkv[:, DH:2 * DH].astype(jnp.bfloat16)
                vs[t] = qkv[:, 2 * DH:].astype(jnp.bfloat16)
            h = t - 1
            if 0 <= h < H:
                ss[h] = _dot(qs[h], ks[h], _NT)
            h = t - 2
            if 0 <= h < H:
                s = jnp.where(mask, ss[h] * (DH ** -0.5), NEG)
                p = jnp.exp(s - jnp.max(s, axis=1, keepdims=True))
                ps[h] = p / jnp.sum(p, axis=1, keepdims=True)
            h = t - 3
            if 0 <= h < H:
                os_[h] = _dot(ps[h], vs[h])
            h = t - 4
            if 0 <= h < H:
                d = _dot(os_[h], wao[pl.ds(h * DM, DM), :], _NT)
                acc = d if acc is None else acc + d
        out[pl.ds(r0, seg), pl.ds(0, DM)] = acc[MEM:].astype(jnp.bfloat16)
        return acc[:MEM].astype(jnp.bfloat16).astype(jnp.float32)
    lax.fori_loop(0, S // seg, a_body, mem0[...].astype(jnp.float32))

    TO = 256
    cps = []
    for m in range(S // TO):
        acc = None
        for h in range(H):
            ctx = pltpu.bitcast(qc[h, pl.ds(m * TO // 2, TO // 2), :], jnp.bfloat16)
            d = _dot(wbo[pl.ds(h * DM, DM), :], ctx, _NT)
            acc = d if acc is None else acc + d
        rows = pl.ds(m * TO, TO)
        out[rows, pl.ds(DM, DM)] = acc.astype(jnp.bfloat16).T
        cp = pltpu.make_async_copy(out.at[rows, :], o_hbm.at[rows, :], sems.at[18 + m])
        cp.start()
        cps.append(cp)
    for cp in cps:
        cp.wait()


@functools.partial(jax.jit, static_argnames=("A_seg_len",))
def pallas_concat_heads__memory_aug_recurrent_mem_tr__compressed_kv_cla__prompt_kernel(
    A_x, A_mem0, A_Wq, A_Wk, A_Wv, A_Wo, A_seg_len,
    B_x, B_c_kv, B_w_q, B_w_uk, B_w_uv, B_w_o,
):
    bf16, u32 = jnp.bfloat16, jnp.uint32
    args = (
        A_x.reshape(S, DM).T, A_mem0.reshape(MEM, DM),
        A_Wq.reshape(DM * H, DH), A_Wk.reshape(DM * H, DH), A_Wv.reshape(DM * H, DH),
        A_Wo.transpose(0, 2, 1).reshape(H * DM, DH),
        B_x.reshape(S, DM).T, B_c_kv.reshape(S, DC),
        B_w_q.reshape(DM * H, DH), B_w_uk.reshape(DC * H, DH), B_w_uv.reshape(DC * H, DH),
        B_w_o.transpose(0, 2, 1).reshape(H * DM, DH),
    )
    scratch = [
        pltpu.VMEM((DM, S), bf16),
        pltpu.VMEM((S // 2, DM), u32),
        pltpu.VMEM((MEM, DM), bf16),
        pltpu.VMEM((H * DM, DH), bf16),
        pltpu.VMEM((S, DC), bf16),
        pltpu.VMEM((H * DM, DH), bf16),
        pltpu.VMEM((2, DC * 8, 128), u32),
        pltpu.VMEM((2, DC * 8, 128), u32),
        pltpu.VMEM((2, DM * 8, 128), u32),
        pltpu.VMEM((H, DM // 2, 3 * DH), u32),
        pltpu.VMEM((H, DM // 2, DH), u32),
        pltpu.VMEM((H, DC // 2, 2 * DH), u32),
        pltpu.VMEM((H, S // 2, DH), u32),
        pltpu.VMEM((S // 2, 2 * DH), u32),
        pltpu.VMEM((S, 2 * DM), bf16),
        pltpu.SemaphoreType.DMA((24,)),
    ]
    res = pl.pallas_call(
        functools.partial(_kernel, seg=int(A_seg_len)),
        in_specs=[pl.BlockSpec(memory_space=pl.ANY)] * len(args),
        out_specs=pl.BlockSpec(memory_space=pl.ANY),
        out_shape=jax.ShapeDtypeStruct((S, 2 * DM), bf16),
        scratch_shapes=scratch,
        compiler_params=pltpu.CompilerParams(vmem_limit_bytes=120 << 20),
    )(*args)
    return res.reshape(1, S, 2 * DM)
```

```python
import functools

import jax
import jax.numpy as jnp
from jax import lax
import jax.experimental.pallas as pl
import jax.experimental.pallas.tpu as pltpu

S = 2048
DM = 448
H = 16
DH = 256
DC = 1024
MEM = 8
TQ = 256
HB = 128
TO = 256
QN = 4
KVL = 4
KVU = 2
CH = 64
NEG = -1000000000.0
SCALE = DH ** -0.5

_NN = (((1,), (0,)), ((), ()))
_NT = (((1,), (1,)), ((), ()))
bf16, f32, u32 = jnp.bfloat16, jnp.float32, jnp.uint32


def _dot(a, b, dims=_NN):
    return lax.dot_general(a, b, dims, preferred_element_type=f32)


def _pack(x):
    return pltpu.bitcast(x.astype(bf16), u32)


def _unpack(x):
    return pltpu.bitcast(x, bf16)


def _deinterleave_chunk(raw, dst, lane0, t):
    r0 = t * (CH // 2)
    s0 = t * (CH * 8)
    if not isinstance(t, int):
        r0, s0 = pl.multiple_of(r0, CH // 2), pl.multiple_of(s0, CH * 8)
    for half in range(2):
        src = raw.at[half, pl.ds(s0, CH * 8), :]
        for j in range(8):
            xe = src[pl.ds(j, CH // 2, stride=16), :]
            xo = src[pl.ds(8 + j, CH // 2, stride=16), :]
            lanes = pl.ds(lane0 + 128 * half, 128)
            dst[2 * j, pl.ds(r0, CH // 2), lanes] = (xe & u32(0xFFFF)) | (xo << 16)
            dst[2 * j + 1, pl.ds(r0, CH // 2), lanes] = (xe >> 16) | (xo & u32(0xFFFF0000))
            yield 1


def _chain(*gens):
    for g in gens:
        yield from g


def _merge(*streams):
    gens = [g for g, _ in streams]
    totals = [float(t) for _, t in streams]
    done = [0.0] * len(gens)
    live = list(range(len(gens)))
    while live:
        i = min(live, key=lambda n: done[n] / totals[n])
        try:
            done[i] += next(gens[i])
        except StopIteration:
            live.remove(i)


def _kernel(xa_hbm, mem_hbm, aq_hbm, ak_hbm, av_hbm, ao_hbm,
            xb_hbm, c_hbm, bq_hbm, bk_hbm, bv_hbm, bo_hbm,
            o_hbm,
            xta, xtb, xa, xb, mem0, wao, c, wbo, rawq, rawk, rawv, raw0, raw1, raw2,
            wa, wbq, wbkv, qc, kv, out, sems, *, seg):
    L = MEM + seg

    def raw_copies(hbm, raw, s0):
        u = hbm.bitcast(u32)
        return [pltpu.make_async_copy(u.at[:, pl.ds(128 * i, 128)], raw.at[i], sems.at[s0 + i])
                for i in range(2)]

    cp_xb = [pltpu.make_async_copy(xb_hbm, xtb, sems.at[0])]
    cp_bq = raw_copies(bq_hbm, rawq, 1)
    cp_bkv = ([pltpu.make_async_copy(c_hbm, c, sems.at[3])]
              + raw_copies(bk_hbm, rawk, 4) + raw_copies(bv_hbm, rawv, 6)
              + [pltpu.make_async_copy(xa_hbm, xta, sems.at[8])])
    cp_aqk = raw_copies(aq_hbm, raw0, 9) + raw_copies(ak_hbm, raw1, 11)
    cp_a = (raw_copies(av_hbm, raw2, 13)
            + [pltpu.make_async_copy(mem_hbm, mem0, sems.at[15]),
               pltpu.make_async_copy(ao_hbm, wao, sems.at[16])])
    cp_bo = [pltpu.make_async_copy(bo_hbm, wbo, sems.at[17])]

    def start(cps):
        for cp in cps:
            cp.start()

    def wait(cps):
        for cp in cps:
            cp.wait()

    def transpose_x(xt, xs):
        def body(m, _):
            r = pl.multiple_of(m * 128, 128)
            xs[pl.ds(r, 128), :] = pltpu.bitcast(xt[:, pl.ds(pl.multiple_of(2 * r, 256), 256)].T, u32)
            return 0
        lax.fori_loop(0, S // 256, body, 0)

    def deinterleave(raw, dst, lane0, rows):
        def body(t, _):
            _merge((_deinterleave_chunk(raw, dst, lane0, t), 1))
            return 0
        lax.fori_loop(0, rows // CH, body, 0)

    def b_qproj(u):
        h, m0 = u // QN, (u % QN) * (S // QN // 2)
        w = _unpack(wbq[h])
        for m in range(S // QN // 256):
            rows = pl.ds(pl.multiple_of(m0 + m * 128, 128), 128)
            qc[h, rows, :] = _pack(_dot(_unpack(xb[rows, :]), w) * SCALE)
            yield 512

    def b_kvblock(h, m):
        r = m * 128
        if not isinstance(m, int):
            r = pl.multiple_of(r, 128)
        kv[pl.ds(r, 128), :] = _pack(_dot(c[pl.ds(2 * r, 256), :], _unpack(wbkv[h])))
        yield 2048

    def b_attn(h):
        row = lax.broadcasted_iota(jnp.int32, (HB, HB), 0)
        col = lax.broadcasted_iota(jnp.int32, (HB, HB), 1)
        tri = col <= row
        for i in range(S // TQ):
            n = (i + 1) * TQ - HB
            qrows = pl.ds(i * TQ // 2, TQ // 2)
            q = _unpack(qc[h, qrows, :])
            conv = lambda r0, nr, l0: _unpack(kv[pl.ds(r0 // 2, nr // 2), pl.ds(l0, DH)])
            sa = _dot(q, conv(0, n, 0), _NT)
            sb = _dot(q[HB:], conv(n, HB, 0), _NT)
            yield n + HB // 2
            su = jnp.where(tri, sa[:HB, n - HB:], NEG)
            if i > 0:
                su = jnp.concatenate([sa[:HB, :n - HB], su], axis=1)
            sl = jnp.concatenate([sa[HB:], jnp.where(tri, sb, NEG)], axis=1)
            pu = jnp.exp(su - jnp.max(su, axis=1, keepdims=True))
            pl_ = jnp.exp(sl - jnp.max(sl, axis=1, keepdims=True))
            lu = jnp.sum(pu, axis=1, keepdims=True)
            ll = jnp.sum(pl_, axis=1, keepdims=True)
            pa = jnp.concatenate([pu.astype(bf16), pl_[:, :n].astype(bf16)], axis=0)
            o = _dot(pa, conv(0, n, DH))
            ob = _dot(pl_[:, n:].astype(bf16), conv(n, HB, DH))
            o = jnp.concatenate([o[:HB] / lu, (o[HB:] + ob) / ll], axis=0)
            qc[h, qrows, :] = _pack(o)
            yield n + HB // 2

    def out_copy(m):
        rows = pl.ds(pl.multiple_of(m * TO, TO), TO)
        return pltpu.make_async_copy(out.at[rows, :], o_hbm.at[rows, :], sems.at[18 + m])

    def b_outproj(m, _):
        acc = None
        for h in range(H):
            ctx = _unpack(qc[h, pl.ds(pl.multiple_of(m * (TO // 2), TO // 2), TO // 2), :])
            d = _dot(wbo[pl.ds(h * DM, DM), :], ctx, _NT)
            acc = d if acc is None else acc + d
        out[pl.ds(pl.multiple_of(m * TO, TO), TO), pl.ds(DM, DM)] = acc.astype(bf16).T
        out_copy(m).start()
        return 0

    def a_steps(s0, nsteps, state):
        row = lax.broadcasted_iota(jnp.int32, (L, L), 0)
        col = lax.broadcasted_iota(jnp.int32, (L, L), 1)
        mask = (row < MEM) | (row >= col)
        for ds in range(nsteps):
            r0, p0 = (s0 + ds) * seg, (s0 + ds) * (seg // 2)
            if not isinstance(s0, int):
                r0, p0 = pl.multiple_of(r0, seg), pl.multiple_of(p0, seg // 2)
            hx = jnp.concatenate([state[0], _unpack(xa[pl.ds(p0, seg // 2), :]).astype(f32)], axis=0)
            qs, ks, vs, ss, ps, os_ = {}, {}, {}, {}, {}, {}
            acc = None
            for t in range(H + 4):
                cost = 0
                if t < H:
                    qkv = _dot(hx, _unpack(wa[t]))
                    qs[t] = qkv[:, :DH]
                    ks[t] = qkv[:, DH:2 * DH].astype(bf16)
                    vs[t] = qkv[:, 2 * DH:].astype(bf16)
                    cost += 240
                h = t - 1
                if 0 <= h < H:
                    ss[h] = _dot(qs[h], ks[h], _NT)
                    cost += 20
                h = t - 2
                if 0 <= h < H:
                    s = jnp.where(mask, ss[h] * SCALE, NEG)
                    p = jnp.exp(s - jnp.max(s, axis=1, keepdims=True))
                    ps[h] = p / jnp.sum(p, axis=1, keepdims=True)
                h = t - 3
                if 0 <= h < H:
                    os_[h] = _dot(ps[h], vs[h])
                    cost += 20
                h = t - 4
                if 0 <= h < H:
                    d = _dot(os_[h], wao[pl.ds(h * DM, DM), :], _NT)
                    acc = d if acc is None else acc + d
                    cost += 80
                if t == H + 3:
                    out[pl.ds(r0, seg), pl.ds(0, DM)] = acc[MEM:].astype(bf16)
                    state[0] = acc[:MEM].astype(bf16).astype(f32)
                yield cost

    A_COST, ATT_COST = 5760, 17408
    per_head = S // seg // H
    assert per_head * H * seg == S

    start(cp_xb + cp_bq + cp_bkv + cp_aqk + cp_a + cp_bo)
    wait(cp_xb)
    transpose_x(xtb, xb)
    wait(cp_bq)
    deinterleave(rawq, wbq, 0, DM)

    nq = H * QN
    n_kv, n_a = DC // CH, DM // CH

    def q_body(u, _):
        _merge((b_qproj(u), 1))
        return 0
    lax.fori_loop(0, nq - n_kv - n_a, q_body, 0)
    wait(cp_bkv)
    transpose_x(xta, xa)

    def q2_body(t, _):
        de = _chain(_deinterleave_chunk(rawk, wbkv, 0, t), _deinterleave_chunk(rawv, wbkv, DH, t))
        _merge((b_qproj(nq - n_kv - n_a + t), 4096 // QN), (de, 32))
        return 0
    lax.fori_loop(0, n_kv, q2_body, 0)
    wait(cp_aqk)

    def q3_body(t, _):
        de = _chain(_deinterleave_chunk(raw0, wa, 0, t), _deinterleave_chunk(raw1, wa, DH, t))
        _merge((b_qproj(nq - n_a + t), 4096 // QN), (de, 32))
        return 0
    lax.fori_loop(0, n_a, q3_body, 0)
    wait(cp_a)
    deinterleave(raw2, wa, 2 * DH, DM)

    def head_body(h, mem):
        def kv_body(t, _):
            _merge((_chain(*[b_kvblock(h, t * KVU + m) for m in range(KVU)]), 1))
            return 0
        lax.fori_loop(0, KVL // KVU, kv_body, 0)
        state = [mem]
        nf = S // 256 - KVL
        _merge((a_steps(h * per_head, per_head, state), per_head * A_COST),
               (_chain(*[b_kvblock(h, m) for m in range(KVL, S // 256)], b_attn(h)),
                nf * 2048 + ATT_COST))
        return state[0]
    lax.fori_loop(0, H, head_body, mem0[...].astype(f32))

    wait(cp_bo)
    lax.fori_loop(0, S // TO, b_outproj, 0)
    wait([out_copy(m) for m in range(S // TO)])


@functools.partial(jax.jit, static_argnames=("A_seg_len",))
def pallas_concat_heads__memory_aug_recurrent_mem_tr__compressed_kv_cla__prompt_kernel(
    A_x, A_mem0, A_Wq, A_Wk, A_Wv, A_Wo, A_seg_len,
    B_x, B_c_kv, B_w_q, B_w_uk, B_w_uv, B_w_o,
):
    args = (
        A_x.reshape(S, DM).T, A_mem0.reshape(MEM, DM),
        A_Wq.reshape(DM * H, DH), A_Wk.reshape(DM * H, DH), A_Wv.reshape(DM * H, DH),
        A_Wo.transpose(0, 2, 1).reshape(H * DM, DH),
        B_x.reshape(S, DM).T, B_c_kv.reshape(S, DC),
        B_w_q.reshape(DM * H, DH), B_w_uk.reshape(DC * H, DH), B_w_uv.reshape(DC * H, DH),
        B_w_o.transpose(0, 2, 1).reshape(H * DM, DH),
    )
    scratch = [
        pltpu.VMEM((DM, S), bf16),
        pltpu.VMEM((DM, S), bf16),
        pltpu.VMEM((S // 2, DM), u32),
        pltpu.VMEM((S // 2, DM), u32),
        pltpu.VMEM((MEM, DM), bf16),
        pltpu.VMEM((H * DM, DH), bf16),
        pltpu.VMEM((S, DC), bf16),
        pltpu.VMEM((H * DM, DH), bf16),
        pltpu.VMEM((2, DM * 8, 128), u32),
        pltpu.VMEM((2, DC * 8, 128), u32),
        pltpu.VMEM((2, DC * 8, 128), u32),
        pltpu.VMEM((2, DM * 8, 128), u32),
        pltpu.VMEM((2, DM * 8, 128), u32),
        pltpu.VMEM((2, DM * 8, 128), u32),
        pltpu.VMEM((H, DM // 2, 3 * DH), u32),
        pltpu.VMEM((H, DM // 2, DH), u32),
        pltpu.VMEM((H, DC // 2, 2 * DH), u32),
        pltpu.VMEM((H, S // 2, DH), u32),
        pltpu.VMEM((S // 2, 2 * DH), u32),
        pltpu.VMEM((S, 2 * DM), bf16),
        pltpu.SemaphoreType.DMA((18 + S // TO,)),
    ]
    res = pl.pallas_call(
        functools.partial(_kernel, seg=int(A_seg_len)),
        in_specs=[pl.BlockSpec(memory_space=pl.ANY)] * len(args),
        out_specs=pl.BlockSpec(memory_space=pl.ANY),
        out_shape=jax.ShapeDtypeStruct((S, 2 * DM), bf16),
        scratch_shapes=scratch,
        compiler_params=pltpu.CompilerParams(vmem_limit_bytes=120 << 20),
    )(*args)
    return res.reshape(1, S, 2 * DM)
```

```python
import functools

import jax
import jax.numpy as jnp
from jax import lax
import jax.experimental.pallas as pl
import jax.experimental.pallas.tpu as pltpu

S = 2048
DM = 448
H = 16
DH = 256
DC = 1024
MEM = 8
TQ = 256
HB = 128
QORDER = (1, 2, 3, 7, 6, 5, 4, 0)
OSPLIT = 3
RG = 32
ACOST = [280] * 16 + [320] * 4
ALEAD = 1.03
QN = 4
KVL = 6
KVS = 5
KVU = 2
CH = 64
NEG = -1000000000.0
SCALE = DH ** -0.5

_NN = (((1,), (0,)), ((), ()))
_NT = (((1,), (1,)), ((), ()))
bf16, f32, u32 = jnp.bfloat16, jnp.float32, jnp.uint32


def _dot(a, b, dims=_NN):
    return lax.dot_general(a, b, dims, preferred_element_type=f32)


def _pack(x):
    return pltpu.bitcast(x.astype(bf16), u32)


def _unpack(x):
    return pltpu.bitcast(x, bf16)


def _deinterleave_chunk(raw, dst, lane0, t):
    r0 = t * (CH // 2)
    s0 = t * (CH * 8)
    if not isinstance(t, int):
        r0, s0 = pl.multiple_of(r0, CH // 2), pl.multiple_of(s0, CH * 8)
    for half in range(2):
        src = raw.at[half, pl.ds(s0, CH * 8), :]
        for j in range(8):
            xe = src[pl.ds(j, CH // 2, stride=16), :]
            xo = src[pl.ds(8 + j, CH // 2, stride=16), :]
            lanes = pl.ds(lane0 + 128 * half, 128)
            dst[2 * j, pl.ds(r0, CH // 2), lanes] = (xe & u32(0xFFFF)) | (xo << 16)
            dst[2 * j + 1, pl.ds(r0, CH // 2), lanes] = (xe >> 16) | (xo & u32(0xFFFF0000))
            yield 1


def _chain(*gens):
    for g in gens:
        yield from g


def _zip(main, total, side, count):
    done, n = 0.0, 0
    for cst in main:
        done += cst
        while n < count and n < done / total * count:
            next(side)
            n += 1
        yield cst
    for _ in side:
        pass


def _merge(*streams):
    gens = [g for g, _ in streams]
    totals = [float(t) for _, t in streams]
    done = [0.0] * len(gens)
    live = list(range(len(gens)))
    while live:
        i = min(live, key=lambda n: done[n] / totals[n])
        try:
            done[i] += next(gens[i])
        except StopIteration:
            live.remove(i)


def _kernel(xa_hbm, mem_hbm, aq_hbm, ak_hbm, av_hbm, ao_hbm,
            xb_hbm, c_hbm, bq_hbm, bk_hbm, bv_hbm, bo_hbm,
            o_hbm,
            xta, xtb, xa, xb, mem0, wao, c, wbo, rawq, rawk, rawv, raw0, raw1, raw2,
            wa, wbq, wbkv, qc, kv, ot, out, sems, *, seg):
    L = MEM + seg

    def raw_copies(hbm, raw, s0):
        u = hbm.bitcast(u32)
        return [pltpu.make_async_copy(u.at[:, pl.ds(128 * i, 128)], raw.at[i], sems.at[s0 + i])
                for i in range(2)]

    cp_xb = [pltpu.make_async_copy(xb_hbm, xtb, sems.at[0])]
    cp_bq = raw_copies(bq_hbm, rawq, 1)
    cp_bkv = ([pltpu.make_async_copy(c_hbm, c, sems.at[3])]
              + raw_copies(bk_hbm, rawk, 4) + raw_copies(bv_hbm, rawv, 6)
              + [pltpu.make_async_copy(xa_hbm, xta, sems.at[8])])
    cp_aqk = raw_copies(aq_hbm, raw0, 9) + raw_copies(ak_hbm, raw1, 11)
    cp_a = (raw_copies(av_hbm, raw2, 13)
            + [pltpu.make_async_copy(mem_hbm, mem0, sems.at[15]),
               pltpu.make_async_copy(ao_hbm, wao, sems.at[16])])
    cp_bo = [pltpu.make_async_copy(bo_hbm, wbo, sems.at[17])]

    def start(cps):
        for cp in cps:
            cp.start()

    def wait(cps):
        for cp in cps:
            cp.wait()

    def transpose_x(xt, xs):
        def body(m, _):
            r = pl.multiple_of(m * 128, 128)
            xs[pl.ds(r, 128), :] = pltpu.bitcast(xt[:, pl.ds(pl.multiple_of(2 * r, 256), 256)].T, u32)
            return 0
        lax.fori_loop(0, S // 256, body, 0)

    def deinterleave(raw, dst, lane0, rows):
        def body(t, _):
            _merge((_deinterleave_chunk(raw, dst, lane0, t), 1))
            return 0
        lax.fori_loop(0, rows // CH, body, 0)

    def b_qproj(u):
        h, m0 = u // QN, (u % QN) * (S // QN // 2)
        w = _unpack(wbq[h])
        for m in range(S // QN // 256):
            rows = pl.ds(pl.multiple_of(m0 + m * 128, 128), 128)
            qc[h, rows, :] = _pack(_dot(_unpack(xb[rows, :]), w) * SCALE)
            yield 512

    def b_kvblock(h, m):
        r = m * 128
        if not isinstance(m, int):
            r = pl.multiple_of(r, 128)
        for l0 in (0, DH):
            acc = None
            for k0 in range(0, DC, 512):
                d = _dot(c[pl.ds(2 * r, 256), pl.ds(k0, 512)],
                         _unpack(wbkv[h, pl.ds(k0 // 2, 256), pl.ds(l0, DH)]))
                acc = d if acc is None else acc + d
                if k0 + 512 == DC:
                    kv[pl.ds(r, 128), pl.ds(l0, DH)] = _pack(acc)
                yield 512

    def b_attn(h, fill):
        row = lax.broadcasted_iota(jnp.int32, (HB, HB), 0)
        col = lax.broadcasted_iota(jnp.int32, (HB, HB), 1)
        tri = col <= row
        conv = lambda r0, nr, l0: _unpack(kv[pl.ds(r0 // 2, nr // 2), pl.ds(l0, DH)])

        def blocks(i):
            return [(j * TQ, TQ) for j in range(i)] + [(i * TQ, HB)]

        def scores(i, st):
            q = _unpack(qc[h, pl.ds(i * TQ // 2, TQ // 2), :])
            st["s"] = []
            for k0, nk in blocks(i):
                st["s"].append(_dot(q, conv(k0, nk, 0), _NT))
                yield nk
            st["sb"] = _dot(q[HB:], conv(i * TQ + HB, HB, 0), _NT)
            yield HB // 2

        def softmax(i, st):
            st["p"], st["pb"], st["l"] = [], [], []
            for r in range(0, TQ, RG):
                parts = [x[r:r + RG] for x in st["s"]]
                if r < HB:
                    parts[-1] = jnp.where(tri[r:r + RG], parts[-1], NEG)
                else:
                    parts.append(jnp.where(tri[r - HB:r - HB + RG], st["sb"][r - HB:r - HB + RG], NEG))
                s = jnp.concatenate(parts, axis=1)
                p = jnp.exp(s - jnp.max(s, axis=1, keepdims=True))
                st["l"].append(jnp.sum(p, axis=1, keepdims=True))
                p = p.astype(bf16)
                n = i * TQ + HB
                st["p"].append(p[:, :n])
                if r >= HB:
                    st["pb"].append(p[:, n:])
                yield 0

        def values(i, st):
            o = None
            for k0, nk in blocks(i):
                d = _dot(jnp.concatenate([x[:, k0:k0 + nk] for x in st["p"]], axis=0), conv(k0, nk, DH))
                o = d if o is None else o + d
                yield nk
            ob = _dot(jnp.concatenate(st["pb"], axis=0), conv(i * TQ + HB, HB, DH))
            o = jnp.concatenate([o[:HB], o[HB:] + ob], axis=0) / jnp.concatenate(st["l"], axis=0)
            qc[h, pl.ds(i * TQ // 2, TQ // 2), :] = _pack(o)
            yield HB // 2

        cost = lambda i: i * TQ + HB + HB // 2
        sts = [{} for _ in QORDER]
        for t in range(len(QORDER) + 2):
            mxu, tot = [], 0
            if t in fill:
                mxu.append(fill[t][0])
                tot += fill[t][1]
            if t >= 2:
                mxu.append(values(QORDER[t - 2], sts[t - 2]))
                tot += cost(QORDER[t - 2])
            if t < len(QORDER):
                mxu.append(scores(QORDER[t], sts[t]))
                tot += cost(QORDER[t])
            if 1 <= t <= len(QORDER):
                yield from _zip(_chain(*mxu), tot, softmax(QORDER[t - 1], sts[t - 1]), TQ // RG)
            else:
                yield from _chain(*mxu)

    def out_copy(m):
        rows = pl.ds(m * TQ, TQ)
        return pltpu.make_async_copy(out.at[rows, :], o_hbm.at[rows, :], sems.at[18 + m])

    def b_outproj_acc(h, blocks):
        for m in blocks:
            ctx = _unpack(qc[h, pl.ds(m * TQ // 2, TQ // 2), :])
            w = wbo[pl.ds(pl.multiple_of(h * DM, DM), DM), :]
            ot[:, pl.ds(m * TQ, TQ)] += _dot(w, ctx, _NT)
            yield DM

    def emit_block(m, acc):
        out[pl.ds(m * TQ, TQ), pl.ds(DM, DM)] = acc.astype(bf16).T
        out_copy(m).start()

    def b_outproj_last(m):
        acc = None
        for h in range(H):
            ctx = _unpack(qc[h, pl.ds(m * TQ // 2, TQ // 2), :])
            d = _dot(wbo[pl.ds(h * DM, DM), :], ctx, _NT)
            acc = d if acc is None else acc + d
            yield 2
        emit_block(m, acc)

    def emit_blocks(blocks):
        for m in blocks:
            emit_block(m, ot[:, pl.ds(m * TQ, TQ)])
            yield 1

    def a_steps(s0, nsteps, state):
        row = lax.broadcasted_iota(jnp.int32, (L, L), 0)
        col = lax.broadcasted_iota(jnp.int32, (L, L), 1)
        mask = (row < MEM) | (row >= col)
        for ds in range(nsteps):
            r0, p0 = (s0 + ds) * seg, (s0 + ds) * (seg // 2)
            if not isinstance(s0, int):
                r0, p0 = pl.multiple_of(r0, seg), pl.multiple_of(p0, seg // 2)
            hx = jnp.concatenate([state[0], _unpack(xa[pl.ds(p0, seg // 2), :]).astype(f32)], axis=0)
            qs, ks, vs, ss, ps, os_ = {}, {}, {}, {}, {}, {}
            acc = None
            for t in range(H + 4):
                cost = 0
                if t < H:
                    qkv = _dot(hx, _unpack(wa[t]))
                    qs[t] = qkv[:, :DH]
                    ks[t] = qkv[:, DH:2 * DH].astype(bf16)
                    vs[t] = qkv[:, 2 * DH:].astype(bf16)
                    cost += 240
                h = t - 1
                if 0 <= h < H:
                    ss[h] = _dot(qs[h], ks[h], _NT)
                    cost += 20
                h = t - 2
                if 0 <= h < H:
                    s = jnp.where(mask, ss[h] * SCALE, NEG)
                    p = jnp.exp(s - jnp.max(s, axis=1, keepdims=True))
                    ps[h] = p / jnp.sum(p, axis=1, keepdims=True)
                h = t - 3
                if 0 <= h < H:
                    os_[h] = _dot(ps[h], vs[h])
                    cost += 20
                h = t - 4
                if 0 <= h < H:
                    d = _dot(os_[h], wao[pl.ds(h * DM, DM), :], _NT)
                    acc = d if acc is None else acc + d
                    cost += 80
                if t == H + 3:
                    out[pl.ds(r0, seg), pl.ds(0, DM)] = acc[MEM:].astype(bf16)
                    state[0] = acc[:MEM].astype(bf16).astype(f32)
                yield ACOST[t]

    A_COST, ATT_COST = 5760, 17408
    per_head = S // seg // H
    assert per_head * H * seg == S

    start(cp_xb + cp_bq + cp_bkv + cp_aqk + cp_a + cp_bo)
    ot[...] = jnp.zeros_like(ot)
    wait(cp_xb)
    transpose_x(xtb, xb)
    wait(cp_bq)
    deinterleave(rawq, wbq, 0, DM)

    nq = H * QN
    n_kv, n_a = DC // CH, DM // CH

    def q_body(u, _):
        _merge((b_qproj(u), 1))
        return 0
    lax.fori_loop(0, nq - n_kv - n_a, q_body, 0)
    wait(cp_bkv)
    transpose_x(xta, xa)

    def q2_body(t, _):
        de = _chain(_deinterleave_chunk(rawk, wbkv, 0, t), _deinterleave_chunk(rawv, wbkv, DH, t))
        _merge((b_qproj(nq - n_kv - n_a + t), 4096 // QN), (de, 32))
        return 0
    lax.fori_loop(0, n_kv, q2_body, 0)
    wait(cp_aqk)

    def q3_body(t, _):
        de = _chain(_deinterleave_chunk(raw0, wa, 0, t), _deinterleave_chunk(raw1, wa, DH, t))
        _merge((b_qproj(nq - n_a + t), 4096 // QN), (de, 32))
        return 0
    lax.fori_loop(0, n_a, q3_body, 0)
    wait(cp_a)
    deinterleave(raw2, wa, 2 * DH, DM)

    nb = S // TQ

    def head_body(h, mem):
        def kv_body(t, _):
            _merge((_chain(*[b_kvblock(h, t * KVU + m) for m in range(KVU)]), 1))
            return 0
        lax.fori_loop(0, KVL // KVU, kv_body, 0)
        state = [mem]
        nf = S // 256 - KVL
        fill = {m - KVS: (b_kvblock(h, m), 2048) for m in range(KVL, S // 256)}
        fill[nb] = (b_outproj_acc(h, QORDER[:OSPLIT]), OSPLIT * DM)
        fill[nb + 1] = (b_outproj_acc(h, QORDER[OSPLIT:-1]), (nb - 1 - OSPLIT) * DM)
        _merge((a_steps(h * per_head, per_head, state), per_head * sum(ACOST) * ALEAD),
               (b_attn(h, fill), nf * 2048 + ATT_COST + (nb - 1) * DM))
        return state[0]
    lax.fori_loop(0, H, head_body, mem0[...].astype(f32))

    wait(cp_bo)
    _merge((emit_blocks(QORDER[:-1]), 3 * (nb - 1)), (b_outproj_last(QORDER[-1]), 3 * H))
    wait([out_copy(m) for m in range(S // TQ)])


@functools.partial(jax.jit, static_argnames=("A_seg_len",))
def pallas_concat_heads__memory_aug_recurrent_mem_tr__compressed_kv_cla__prompt_kernel(
    A_x, A_mem0, A_Wq, A_Wk, A_Wv, A_Wo, A_seg_len,
    B_x, B_c_kv, B_w_q, B_w_uk, B_w_uv, B_w_o,
):
    args = (
        A_x.reshape(S, DM).T, A_mem0.reshape(MEM, DM),
        A_Wq.reshape(DM * H, DH), A_Wk.reshape(DM * H, DH), A_Wv.reshape(DM * H, DH),
        A_Wo.transpose(0, 2, 1).reshape(H * DM, DH),
        B_x.reshape(S, DM).T, B_c_kv.reshape(S, DC),
        B_w_q.reshape(DM * H, DH), B_w_uk.reshape(DC * H, DH), B_w_uv.reshape(DC * H, DH),
        B_w_o.transpose(0, 2, 1).reshape(H * DM, DH),
    )
    scratch = [
        pltpu.VMEM((DM, S), bf16),
        pltpu.VMEM((DM, S), bf16),
        pltpu.VMEM((S // 2, DM), u32),
        pltpu.VMEM((S // 2, DM), u32),
        pltpu.VMEM((MEM, DM), bf16),
        pltpu.VMEM((H * DM, DH), bf16),
        pltpu.VMEM((S, DC), bf16),
        pltpu.VMEM((H * DM, DH), bf16),
        pltpu.VMEM((2, DM * 8, 128), u32),
        pltpu.VMEM((2, DC * 8, 128), u32),
        pltpu.VMEM((2, DC * 8, 128), u32),
        pltpu.VMEM((2, DM * 8, 128), u32),
        pltpu.VMEM((2, DM * 8, 128), u32),
        pltpu.VMEM((2, DM * 8, 128), u32),
        pltpu.VMEM((H, DM // 2, 3 * DH), u32),
        pltpu.VMEM((H, DM // 2, DH), u32),
        pltpu.VMEM((H, DC // 2, 2 * DH), u32),
        pltpu.VMEM((H, S // 2, DH), u32),
        pltpu.VMEM((S // 2, 2 * DH), u32),
        pltpu.VMEM((DM, S), f32),
        pltpu.VMEM((S, 2 * DM), bf16),
        pltpu.SemaphoreType.DMA((18 + S // TQ,)),
    ]
    res = pl.pallas_call(
        functools.partial(_kernel, seg=int(A_seg_len)),
        in_specs=[pl.BlockSpec(memory_space=pl.ANY)] * len(args),
        out_specs=pl.BlockSpec(memory_space=pl.ANY),
        out_shape=jax.ShapeDtypeStruct((S, 2 * DM), bf16),
        scratch_shapes=scratch,
        compiler_params=pltpu.CompilerParams(vmem_limit_bytes=120 << 20),
    )(*args)
    return res.reshape(1, S, 2 * DM)
```

```python
import functools

import jax
import jax.numpy as jnp
from jax import lax
import jax.experimental.pallas as pl
import jax.experimental.pallas.tpu as pltpu

S = 2048
DM = 448
H = 16
DH = 256
DC = 1024
MEM = 8
TQ = 256
HB = 128
QORDER = (1, 2, 3, 7, 6, 5, 4, 0)
OSPLIT = 3
RG = 32
DMM = 384
GROUPS = ((0, 1, 2), (3, 4, 5), (6, 7, 8), (9, 10, 11), (12, 13), (14, 15))
ASCHED = (("p0", 320), ("p1", 320), ("p2 s0", 380), ("p3 s1 f0", 380), ("p4 f1", 320), ("p5 s2", 380), ("p6 s3 f2", 380), ("p7 s4 f3", 360), ("z0 s5 f4", 320), ("z1 f5", 280), ("z2 m0", 320), ("z3 m1", 320), ("z4", 280), ("z5 m2", 320), ("z6 m3", 320), ("z7 m4", 320), ("", 200), ("m5", 300))
ALEAD = 1.03
QN = 2
KVL = 8
KVS = 5
KVU = 2
CH = 64
NEG = -1000000000.0
SCALE = DH ** -0.5

_NN = (((1,), (0,)), ((), ()))
_NT = (((1,), (1,)), ((), ()))
bf16, f32, u32 = jnp.bfloat16, jnp.float32, jnp.uint32


def _dot(a, b, dims=_NN):
    return lax.dot_general(a, b, dims, preferred_element_type=f32)


def _pack(x):
    return pltpu.bitcast(x.astype(bf16), u32)


def _unpack(x):
    return pltpu.bitcast(x, bf16)


def _deinterleave_chunk(raw, dst, place, t):
    r0 = t * (CH // 2)
    s0 = t * (CH * 8)
    if not isinstance(t, int):
        r0, s0 = pl.multiple_of(r0, CH // 2), pl.multiple_of(s0, CH * 8)
    for half in range(2):
        src = raw.at[half, pl.ds(s0, CH * 8), :]
        for j in range(8):
            xe = src[pl.ds(j, CH // 2, stride=16), :]
            xo = src[pl.ds(8 + j, CH // 2, stride=16), :]
            vals = ((xe & u32(0xFFFF)) | (xo << 16), (xe >> 16) | (xo & u32(0xFFFF0000)))
            for e in range(2):
                i, r, l = place(2 * j + e, half)
                dst[i, pl.ds(r + r0, CH // 2), pl.ds(l, 128)] = vals[e]
            yield 1


def _chain(*gens):
    for g in gens:
        yield from g


def _zip(main, total, side, count):
    done, n = 0.0, 0
    for cst in main:
        done += cst
        while n < count and n < done / total * count:
            next(side)
            n += 1
        yield cst
    for _ in side:
        pass


def _merge(*streams):
    gens = [g for g, _ in streams]
    totals = [float(t) for _, t in streams]
    done = [0.0] * len(gens)
    live = list(range(len(gens)))
    while live:
        i = min(live, key=lambda n: done[n] / totals[n])
        try:
            done[i] += next(gens[i])
        except StopIteration:
            live.remove(i)


def _kernel(xa_hbm, mem_hbm, aq_hbm, ak_hbm, av_hbm, ao_hbm,
            xb_hbm, c_hbm, bq_hbm, bk_hbm, bv_hbm, bo_hbm,
            o_hbm,
            xta, xtb, xa, xb, mem0, wao, c, wbo, rawq, rawk, rawv, raw0, raw1, raw2,
            wa, wbq, wbkv, qc, kv, ot, out, sems, *, seg):
    L = MEM + seg

    def raw_copies(hbm, raw, s0):
        u = hbm.bitcast(u32)
        return [pltpu.make_async_copy(u.at[:, pl.ds(128 * i, 128)], raw.at[i], sems.at[s0 + i])
                for i in range(2)]

    cp_xb = [pltpu.make_async_copy(xb_hbm, xtb, sems.at[0])]
    cp_bq = raw_copies(bq_hbm, rawq, 1)
    cp_bkv = ([pltpu.make_async_copy(c_hbm, c, sems.at[3])]
              + raw_copies(bk_hbm, rawk, 4) + raw_copies(bv_hbm, rawv, 6)
              + [pltpu.make_async_copy(xa_hbm, xta, sems.at[8])])
    cp_avo = raw_copies(av_hbm, raw2, 9) + [pltpu.make_async_copy(ao_hbm, wao, sems.at[11])]
    cp_aqk = (raw_copies(aq_hbm, raw0, 12) + raw_copies(ak_hbm, raw1, 14)
              + [pltpu.make_async_copy(mem_hbm, mem0, sems.at[16])])
    cp_bo = [pltpu.make_async_copy(bo_hbm, wbo, sems.at[17])]

    def start(cps):
        for cp in cps:
            cp.start()

    def wait(cps):
        for cp in cps:
            cp.wait()

    def transpose_x(xt, xs, m):
        r = pl.multiple_of(m * 128, 128)
        xs[pl.ds(r, 128), :] = pltpu.bitcast(xt[:, pl.ds(pl.multiple_of(2 * r, 256), 256)].T, u32)
        yield 1

    def deinterleave(raw, dst, place, rows):
        def body(t, _):
            _merge((_deinterleave_chunk(raw, dst, place, t), 1))
            return 0
        lax.fori_loop(0, rows // CH, body, 0)

    def b_qproj(u):
        h, m0 = u // QN, (u % QN) * (S // QN // 2)
        w = _unpack(wbq[h])
        for m in range(S // QN // 256):
            rows = pl.ds(pl.multiple_of(m0 + m * 128, 128), 128)
            qc[h, rows, :] = _pack(_dot(_unpack(xb[rows, :]), w) * SCALE)
            yield 512

    def b_kvblock(h, m):
        r = m * 128
        if not isinstance(m, int):
            r = pl.multiple_of(r, 128)
        for l0 in (0, DH):
            acc = None
            for k0 in range(0, DC, 512):
                d = _dot(c[pl.ds(2 * r, 256), pl.ds(k0, 512)],
                         _unpack(wbkv[h, pl.ds(k0 // 2, 256), pl.ds(l0, DH)]))
                acc = d if acc is None else acc + d
                if k0 + 512 == DC:
                    kv[pl.ds(r, 128), pl.ds(l0, DH)] = _pack(acc)
                yield 512

    def b_attn(h, fill):
        row = lax.broadcasted_iota(jnp.int32, (HB, HB), 0)
        col = lax.broadcasted_iota(jnp.int32, (HB, HB), 1)
        tri = col <= row
        conv = lambda r0, nr, l0: _unpack(kv[pl.ds(r0 // 2, nr // 2), pl.ds(l0, DH)])

        def blocks(i):
            return [(j * TQ, TQ) for j in range(i)] + [(i * TQ, HB)]

        def scores(i, st):
            q = _unpack(qc[h, pl.ds(i * TQ // 2, TQ // 2), :])
            st["s"] = []
            for k0, nk in blocks(i):
                st["s"].append(_dot(q, conv(k0, nk, 0), _NT))
                yield nk
            st["sb"] = _dot(q[HB:], conv(i * TQ + HB, HB, 0), _NT)
            yield HB // 2

        def softmax(i, st):
            st["p"], st["pb"], st["l"] = [], [], []
            for r in range(0, TQ, RG):
                parts = [x[r:r + RG] for x in st["s"]]
                if r < HB:
                    parts[-1] = jnp.where(tri[r:r + RG], parts[-1], NEG)
                else:
                    parts.append(jnp.where(tri[r - HB:r - HB + RG], st["sb"][r - HB:r - HB + RG], NEG))
                s = jnp.concatenate(parts, axis=1)
                p = jnp.exp(s - jnp.max(s, axis=1, keepdims=True))
                st["l"].append(jnp.sum(p, axis=1, keepdims=True))
                p = p.astype(bf16)
                n = i * TQ + HB
                st["p"].append(p[:, :n])
                if r >= HB:
                    st["pb"].append(p[:, n:])
                yield 0

        def values(i, st):
            o = None
            for k0, nk in blocks(i):
                d = _dot(jnp.concatenate([x[:, k0:k0 + nk] for x in st["p"]], axis=0), conv(k0, nk, DH))
                o = d if o is None else o + d
                yield nk
            ob = _dot(jnp.concatenate(st["pb"], axis=0), conv(i * TQ + HB, HB, DH))
            o = jnp.concatenate([o[:HB], o[HB:] + ob], axis=0) / jnp.concatenate(st["l"], axis=0)
            qc[h, pl.ds(i * TQ // 2, TQ // 2), :] = _pack(o)
            yield HB // 2

        cost = lambda i: i * TQ + HB + HB // 2
        sts = [{} for _ in QORDER]
        for t in range(len(QORDER) + 2):
            mxu, tot = [], 0
            if t in fill:
                mxu.append(fill[t][0])
                tot += fill[t][1]
            if t >= 2:
                mxu.append(values(QORDER[t - 2], sts[t - 2]))
                tot += cost(QORDER[t - 2])
            if t < len(QORDER):
                mxu.append(scores(QORDER[t], sts[t]))
                tot += cost(QORDER[t])
            if 1 <= t <= len(QORDER):
                yield from _zip(_chain(*mxu), tot, softmax(QORDER[t - 1], sts[t - 1]), TQ // RG)
            else:
                yield from _chain(*mxu)

    def out_copy(m):
        rows = pl.ds(m * TQ, TQ)
        return pltpu.make_async_copy(out.at[rows, :], o_hbm.at[rows, :], sems.at[18 + m])

    def b_outproj_acc(h, blocks):
        for m in blocks:
            ctx = _unpack(qc[h, pl.ds(m * TQ // 2, TQ // 2), :])
            w = wbo[pl.ds(pl.multiple_of(h * DM, DM), DM), :]
            ot[:, pl.ds(m * TQ, TQ)] += _dot(w, ctx, _NT)
            yield DM

    def emit_block(m, acc):
        out[pl.ds(m * TQ, TQ), pl.ds(DM, DM)] = acc.astype(bf16).T
        out_copy(m).start()

    def b_outproj_last(m):
        acc = None
        for h in range(H):
            ctx = _unpack(qc[h, pl.ds(m * TQ // 2, TQ // 2), :])
            d = _dot(wbo[pl.ds(h * DM, DM), :], ctx, _NT)
            acc = d if acc is None else acc + d
            yield 2
        emit_block(m, acc)

    def emit_blocks(blocks):
        for m in blocks:
            emit_block(m, ot[:, pl.ds(m * TQ, TQ)])
            yield 1

    def a_absorb(j):
        lane = lax.broadcasted_iota(jnp.int32, (DM, 128), 1)
        tails = []
        for e in range(2):
            wrows = pl.ds(pl.multiple_of((2 * j + e) * (DM // 2), 32), DM // 2)
            wv = _unpack(jnp.concatenate([rawq[0, wrows, :], rawq[1, wrows, :]], axis=1))
            r0 = pl.multiple_of((2 * j + e) * DM, 64)
            wa[j, :, pl.ds(4 * DH + e * DMM, DMM)] = _pack(_dot(wv, wao[pl.ds(r0, DMM), :], _NT))
            yield 3
            rt = pl.multiple_of(r0 + DMM - 64 * e, 64)
            tails.append(_dot(wv, wao[pl.ds(rt, 128), :], _NT))
            yield 1
        wa[j, :, pl.ds(4 * DH + 2 * DMM, 128)] = _pack(jnp.where(lane < 64, tails[0], tails[1]))

    def a_steps(s0, nsteps, state):
        row = lax.broadcasted_iota(jnp.int32, (L, 128), 0)
        col = lax.broadcasted_iota(jnp.int32, (L, 128), 1)
        key = col - jnp.where(col >= 2 * L, 2 * L, jnp.where(col >= L, L, 0))
        mask = (row < MEM) | (row >= key)
        seg_of = [(col >= g * L) & (col < (g + 1) * L) for g in range(3)]

        def pick(xs):
            r = xs[-1]
            for g in range(len(xs) - 2, -1, -1):
                r = jnp.where(col < (g + 1) * L, xs[g], r)
            return r

        def stack(xs):
            pad = jnp.zeros((128 - L * len(xs), xs[0].shape[1]), f32)
            return jnp.concatenate(xs + [pad], axis=0).astype(bf16)

        for ds in range(nsteps):
            r0, p0 = (s0 + ds) * seg, (s0 + ds) * (seg // 2)
            r0, p0 = pl.multiple_of(r0, seg), pl.multiple_of(p0, seg // 2)
            hx = jnp.concatenate([state[0], _unpack(xa[pl.ds(p0, seg // 2), :]).astype(f32)], axis=0)
            qs, ks, zs, ss, ps = {}, {}, {}, {}, {}
            acc = [None]

            def project(j):
                qk = _dot(hx, _unpack(wa[j, :, pl.ds(0, 4 * DH)]))
                for e in range(2):
                    qs[2 * j + e] = qk[:, 2 * e * DH:(2 * e + 1) * DH]
                    ks[2 * j + e] = qk[:, (2 * e + 1) * DH:(2 * e + 2) * DH]

            def project_z(j):
                z = _dot(hx, _unpack(wa[j, :, pl.ds(4 * DH, 2 * DMM + 128)]))
                for e in range(2):
                    tail = jnp.where((col < 64) if e == 0 else (col >= 64), z[:, 2 * DMM:], 0.0)
                    zs[2 * j + e] = jnp.concatenate([z[:, e * DMM:(e + 1) * DMM], tail], axis=1)

            def score(g):
                hs = GROUPS[g]
                r = _dot(jnp.concatenate([qs[h] for h in hs], axis=0), stack([ks[h] for h in hs]), _NT)
                ss[g] = pick([r[n * L:(n + 1) * L] for n in range(len(hs))])

            def soft(g):
                n = len(GROUPS[g])
                s = jnp.where(mask, ss[g] * SCALE, NEG)
                m = pick([jnp.max(jnp.where(seg_of[i], s, -jnp.inf), axis=1, keepdims=True) for i in range(n)])
                p = jnp.where(col < n * L, jnp.exp(s - m), 0.0)
                l = pick([jnp.sum(jnp.where(seg_of[i], p, 0.0), axis=1, keepdims=True) for i in range(n)])
                ps[g] = p / l

            def mix(g):
                d = _dot(ps[g], stack([zs[h] for h in GROUPS[g]]))
                acc[0] = d if acc[0] is None else acc[0] + d

            ops = {"p": project, "z": project_z, "s": score, "f": soft, "m": mix}
            for stage, cst in ASCHED:
                for op in stage.split():
                    ops[op[0]](int(op[1]))
                if stage is ASCHED[-1][0]:
                    t = acc[0][:, DMM:]
                    o = jnp.concatenate([acc[0][:, :DMM], (t + pltpu.roll(t, 64, 1))[:, :64]], axis=1)
                    out[pl.ds(r0, seg), pl.ds(0, DM)] = o[MEM:].astype(bf16)
                    state[0] = o[:MEM].astype(bf16).astype(f32)
                yield cst

    ATT_COST = 17408
    per_head = S // seg // H
    assert per_head * H * seg == S and 3 * L <= 128

    start(cp_xb + cp_bq + cp_bkv + cp_avo + cp_aqk + cp_bo)
    ot[...] = jnp.zeros_like(ot)
    wait(cp_xb)

    def xb_body(m, _):
        _merge((transpose_x(xtb, xb, m), 1))
        return 0
    lax.fori_loop(0, S // 256, xb_body, 0)
    wait(cp_bq)
    deinterleave(rawq, wbq, lambda h, e: (h, 0, 128 * e), DM)

    nq = H * QN
    n_kv, n_a = 4, DM // CH
    kvc = DC // CH // n_kv

    def q_body(u, _):
        _merge((b_qproj(u), 1))
        return 0
    lax.fori_loop(0, nq - n_kv - n_a, q_body, 0)
    wait(cp_bkv)

    def q2_body(t, _):
        de = _chain(*[_deinterleave_chunk(raw, wbkv, lambda h, e, l=l: (h, 0, l + 128 * e), t * kvc + i)
                      for i in range(kvc) for raw, l in ((rawk, 0), (rawv, DH))])
        tr = _chain(*[transpose_x(xta, xa, t * 2 + i) for i in range(2)])
        _merge((b_qproj(nq - n_kv - n_a + t), 4096 // QN), (de, 32 * kvc), (tr, 2))
        return 0
    lax.fori_loop(0, n_kv, q2_body, 0)
    wait(cp_avo)

    def q3_body(t, _):
        _merge((b_qproj(nq - n_a + t), 4096 // QN),
               (_deinterleave_chunk(raw2, rawq, lambda h, e: (e, h * (DM // 2), 0), t), 16))
        return 0
    lax.fori_loop(0, n_a, q3_body, 0)
    wait(cp_aqk)

    def absorb_body(j, _):
        t = jnp.minimum(j, n_a - 1)
        de = _chain(*[_deinterleave_chunk(raw, wa, lambda h, e, l=l: (h // 2, 0, (h % 2) * 2 * DH + l + 128 * e), t)
                      for raw, l in ((raw0, 0), (raw1, DH))])
        _merge((a_absorb(j), 8), (de, 32))
        return 0
    lax.fori_loop(0, H // 2, absorb_body, 0)

    nb = S // TQ

    def head_body(h, mem):
        def kv_body(t, _):
            _merge((_chain(*[b_kvblock(h, t * KVU + m) for m in range(KVU)]), 1))
            return 0
        lax.fori_loop(0, KVL // KVU, kv_body, 0)
        state = [mem]
        nf = S // 256 - KVL
        fill = {m - KVS: (b_kvblock(h, m), 2048) for m in range(KVL, S // 256)}
        fill[nb] = (b_outproj_acc(h, QORDER[:OSPLIT]), OSPLIT * DM)
        fill[nb + 1] = (b_outproj_acc(h, QORDER[OSPLIT:-1]), (nb - 1 - OSPLIT) * DM)
        _merge((a_steps(h * per_head, per_head, state), per_head * sum(c_ for _, c_ in ASCHED) * ALEAD),
               (b_attn(h, fill), nf * 2048 + ATT_COST + (nb - 1) * DM))
        return state[0]
    wait(cp_bo)
    lax.fori_loop(0, H, head_body, mem0[...].astype(f32))

    _merge((emit_blocks(QORDER[:-1]), 3 * (nb - 1)), (b_outproj_last(QORDER[-1]), 3 * H))
    wait([out_copy(m) for m in range(S // TQ)])


@functools.partial(jax.jit, static_argnames=("A_seg_len",))
def pallas_concat_heads__memory_aug_recurrent_mem_tr__compressed_kv_cla__prompt_kernel(
    A_x, A_mem0, A_Wq, A_Wk, A_Wv, A_Wo, A_seg_len,
    B_x, B_c_kv, B_w_q, B_w_uk, B_w_uv, B_w_o,
):
    args = (
        A_x.reshape(S, DM).T, A_mem0.reshape(MEM, DM),
        A_Wq.reshape(DM * H, DH), A_Wk.reshape(DM * H, DH), A_Wv.reshape(DM * H, DH),
        A_Wo.transpose(0, 2, 1).reshape(H * DM, DH),
        B_x.reshape(S, DM).T, B_c_kv.reshape(S, DC),
        B_w_q.reshape(DM * H, DH), B_w_uk.reshape(DC * H, DH), B_w_uv.reshape(DC * H, DH),
        B_w_o.transpose(0, 2, 1).reshape(H * DM, DH),
    )
    scratch = [
        pltpu.VMEM((DM, S), bf16),
        pltpu.VMEM((DM, S), bf16),
        pltpu.VMEM((S // 2, DM), u32),
        pltpu.VMEM((S // 2, DM), u32),
        pltpu.VMEM((MEM, DM), bf16),
        pltpu.VMEM((H * DM, DH), bf16),
        pltpu.VMEM((S, DC), bf16),
        pltpu.VMEM((H * DM, DH), bf16),
        pltpu.VMEM((2, DM * 8, 128), u32),
        pltpu.VMEM((2, DC * 8, 128), u32),
        pltpu.VMEM((2, DC * 8, 128), u32),
        pltpu.VMEM((2, DM * 8, 128), u32),
        pltpu.VMEM((2, DM * 8, 128), u32),
        pltpu.VMEM((2, DM * 8, 128), u32),
        pltpu.VMEM((H // 2, DM // 2, 4 * DH + 2 * DMM + 128), u32),
        pltpu.VMEM((H, DM // 2, DH), u32),
        pltpu.VMEM((H, DC // 2, 2 * DH), u32),
        pltpu.VMEM((H, S // 2, DH), u32),
        pltpu.VMEM((S // 2, 2 * DH), u32),
        pltpu.VMEM((DM, S), f32),
        pltpu.VMEM((S, 2 * DM), bf16),
        pltpu.SemaphoreType.DMA((18 + S // TQ,)),
    ]
    res = pl.pallas_call(
        functools.partial(_kernel, seg=int(A_seg_len)),
        in_specs=[pl.BlockSpec(memory_space=pl.ANY)] * len(args),
        out_specs=pl.BlockSpec(memory_space=pl.ANY),
        out_shape=jax.ShapeDtypeStruct((S, 2 * DM), bf16),
        scratch_shapes=scratch,
        compiler_params=pltpu.CompilerParams(vmem_limit_bytes=120 << 20),
    )(*args)
    return res.reshape(1, S, 2 * DM)
```

```python
import functools

import jax
import jax.numpy as jnp
from jax import lax
import jax.experimental.pallas as pl
import jax.experimental.pallas.tpu as pltpu

S = 2048
DM = 448
H = 16
DH = 256
DC = 1024
MEM = 8
TQ = 256
HB = 128
QORDER = (1, 2, 3, 7, 6, 5, 4, 0)
OSPLIT = 3
RG = 32
DMM = 384
GROUPS = ((0, 1, 2), (3, 4, 5), (6, 7, 8), (9, 10, 11), (12, 13), (14, 15))
ASCHED = (("p0", 320), ("p1", 320), ("p2 s0", 380), ("p3 s1 f0", 380), ("p4 f1", 320), ("p5 s2", 380), ("p6 s3 f2", 380), ("p7 s4 f3", 360), ("z0 s5 f4", 320), ("z1 f5", 280), ("z2 m0", 320), ("z3 m1", 320), ("z4", 280), ("z5 m2", 320), ("z6 m3", 320), ("z7 m4", 320), ("", 200), ("m5", 300))
ALEAD = 1.1
QN = 2
CH = 64
NEG = -1000000000.0
SCALE = DH ** -0.5

_NN = (((1,), (0,)), ((), ()))
_NT = (((1,), (1,)), ((), ()))
bf16, f32, u32 = jnp.bfloat16, jnp.float32, jnp.uint32


def _dot(a, b, dims=_NN):
    return lax.dot_general(a, b, dims, preferred_element_type=f32)


def _pack(x):
    return pltpu.bitcast(x.astype(bf16), u32)


def _unpack(x):
    return pltpu.bitcast(x, bf16)


def _deinterleave_chunk(raw, dst, place, t):
    r0 = t * (CH // 2)
    s0 = t * (CH * 8)
    if not isinstance(t, int):
        r0, s0 = pl.multiple_of(r0, CH // 2), pl.multiple_of(s0, CH * 8)
    for half in range(2):
        src = raw.at[half, pl.ds(s0, CH * 8), :]
        for j in range(8):
            xe = src[pl.ds(j, CH // 2, stride=16), :]
            xo = src[pl.ds(8 + j, CH // 2, stride=16), :]
            vals = ((xe & u32(0xFFFF)) | (xo << 16), (xe >> 16) | (xo & u32(0xFFFF0000)))
            for e in range(2):
                i, r, l = place(2 * j + e, half)
                dst[i, pl.ds(r + r0, CH // 2), pl.ds(l, 128)] = vals[e]
            yield 1


def _chain(*gens):
    for g in gens:
        yield from g


def _zip(main, total, side, count):
    done, n = 0.0, 0
    for cst in main:
        done += cst
        while n < count and n < done / total * count:
            next(side)
            n += 1
        yield cst
    for _ in side:
        pass


def _merge(*streams):
    gens = [g for g, _ in streams]
    totals = [float(t) for _, t in streams]
    done = [0.0] * len(gens)
    live = list(range(len(gens)))
    while live:
        i = min(live, key=lambda n: done[n] / totals[n])
        try:
            done[i] += next(gens[i])
        except StopIteration:
            live.remove(i)


def _kernel(xa_hbm, mem_hbm, aq_hbm, ak_hbm, av_hbm, ao_hbm,
            xb_hbm, c_hbm, bq_hbm, bk_hbm, bv_hbm, bo_hbm,
            o_hbm,
            xta, xtb, xa, xb, mem0, wao, c, wbo, rawq, rawkv, raw0, raw1, raw2,
            wa, wbq, wbkv, qc, kv, ot, out, sems, *, seg):
    L = MEM + seg

    def raw_copies(hbm, raw, s0):
        u = hbm.bitcast(u32)
        return [pltpu.make_async_copy(u.at[:, pl.ds(128 * i, 128)], raw.at[i], sems.at[s0 + i])
                for i in range(2)]

    half = S // QN

    def xb_copy(i):
        cols = pl.ds(i * half, half)
        return [pltpu.make_async_copy(xb_hbm.at[:, cols], xtb.at[:, cols], sems.at[i])]

    cp_bq = raw_copies(bq_hbm, rawq, 2)
    cp_bk = raw_copies(bk_hbm, rawkv.at[0], 4)
    cp_bv = raw_copies(bv_hbm, rawkv.at[1], 6)
    cp_av = raw_copies(av_hbm, raw2, 8)
    cp_a = ([pltpu.make_async_copy(ao_hbm, wao, sems.at[10]),
             pltpu.make_async_copy(xa_hbm, xta, sems.at[11])]
            + raw_copies(aq_hbm, raw0, 12) + raw_copies(ak_hbm, raw1, 14))
    cp_last = [pltpu.make_async_copy(mem_hbm, mem0, sems.at[16]),
               pltpu.make_async_copy(c_hbm, c, sems.at[17]),
               pltpu.make_async_copy(bo_hbm, wbo, sems.at[18])]

    def start(cps):
        for cp in cps:
            cp.start()

    def wait(cps):
        for cp in cps:
            cp.wait()

    def transpose_x(xt, xs, m):
        r = pl.multiple_of(m * 128, 128)
        xs[pl.ds(r, 128), :] = pltpu.bitcast(xt[:, pl.ds(pl.multiple_of(2 * r, 256), 256)].T, u32)
        yield 1

    def deinterleave(raw, dst, place, rows):
        def body(t, _):
            _merge((_deinterleave_chunk(raw, dst, place, t), 1))
            return 0
        lax.fori_loop(0, rows // CH, body, 0)

    def b_qproj(u):
        h, m0 = u % H, (u // H) * (S // QN // 2)
        w = _unpack(wbq[h])
        for m in range(S // QN // 256):
            rows = pl.ds(pl.multiple_of(m0 + m * 128, 128), 128)
            qc[h, rows, :] = _pack(_dot(_unpack(xb[rows, :]), w) * SCALE)
            yield 512

    def b_kvblock(h, m):
        r = m * 128
        if not isinstance(m, int):
            r = pl.multiple_of(r, 128)
        for l0 in (0, DH):
            acc = None
            for k0 in range(0, DC, 512):
                d = _dot(c[pl.ds(2 * r, 256), pl.ds(k0, 512)],
                         _unpack(wbkv[(l0 // DH) * H + h, pl.ds(k0 // 2, 256), :]))
                acc = d if acc is None else acc + d
                if k0 + 512 == DC:
                    kv[pl.ds(r, 128), pl.ds(l0, DH)] = _pack(acc)
                yield 512

    def b_attn(h, fill):
        row = lax.broadcasted_iota(jnp.int32, (HB, HB), 0)
        col = lax.broadcasted_iota(jnp.int32, (HB, HB), 1)
        tri = col <= row
        conv = lambda r0, nr, l0: _unpack(kv[pl.ds(r0 // 2, nr // 2), pl.ds(l0, DH)])

        def blocks(i):
            return [(j * TQ, TQ) for j in range(i)] + [(i * TQ, HB)]

        def scores(i, st):
            q = _unpack(qc[h, pl.ds(i * TQ // 2, TQ // 2), :])
            st["s"] = []
            for k0, nk in blocks(i):
                st["s"].append(_dot(q, conv(k0, nk, 0), _NT))
                yield nk
            st["sb"] = _dot(q[HB:], conv(i * TQ + HB, HB, 0), _NT)
            yield HB // 2

        def softmax(i, st):
            st["p"], st["pb"], st["l"] = [], [], []
            for r in range(0, TQ, RG):
                parts = [x[r:r + RG] for x in st["s"]]
                if r < HB:
                    parts[-1] = jnp.where(tri[r:r + RG], parts[-1], NEG)
                else:
                    parts.append(jnp.where(tri[r - HB:r - HB + RG], st["sb"][r - HB:r - HB + RG], NEG))
                s = jnp.concatenate(parts, axis=1)
                p = jnp.exp(s - jnp.max(s, axis=1, keepdims=True))
                st["l"].append(jnp.sum(p, axis=1, keepdims=True))
                p = p.astype(bf16)
                n = i * TQ + HB
                st["p"].append(p[:, :n])
                if r >= HB:
                    st["pb"].append(p[:, n:])
                yield 0

        def values(i, st):
            o = None
            for k0, nk in blocks(i):
                d = _dot(jnp.concatenate([x[:, k0:k0 + nk] for x in st["p"]], axis=0), conv(k0, nk, DH))
                o = d if o is None else o + d
                yield nk
            ob = _dot(jnp.concatenate(st["pb"], axis=0), conv(i * TQ + HB, HB, DH))
            o = jnp.concatenate([o[:HB], o[HB:] + ob], axis=0) / jnp.concatenate(st["l"], axis=0)
            qc[h, pl.ds(i * TQ // 2, TQ // 2), :] = _pack(o)
            yield HB // 2

        cost = lambda i: i * TQ + HB + HB // 2
        sts = [{} for _ in QORDER]
        for t in range(len(QORDER) + 2):
            mxu, tot = [], 0
            if t in fill:
                mxu.append(fill[t][0])
                tot += fill[t][1]
            if t >= 2:
                mxu.append(values(QORDER[t - 2], sts[t - 2]))
                tot += cost(QORDER[t - 2])
            if t < len(QORDER):
                mxu.append(scores(QORDER[t], sts[t]))
                tot += cost(QORDER[t])
            if 1 <= t <= len(QORDER):
                yield from _zip(_chain(*mxu), tot, softmax(QORDER[t - 1], sts[t - 1]), TQ // RG)
            else:
                yield from _chain(*mxu)

    def out_copy(m):
        rows, lanes = pl.ds(m * TQ, TQ), pl.ds(DMM, 2 * DM - DMM)
        return pltpu.make_async_copy(out.at[rows, lanes], o_hbm.at[rows, lanes], sems.at[19 + m])

    def out_copy_a(h):
        n = S // H
        rows, lanes = pl.ds(pl.multiple_of(h * n, n), n), pl.ds(0, DMM)
        return pltpu.make_async_copy(out.at[rows, lanes], o_hbm.at[rows, lanes], sems.at[19 + S // TQ])

    def b_outproj_acc(h, blocks):
        for m in blocks:
            ctx = _unpack(qc[h, pl.ds(m * TQ // 2, TQ // 2), :])
            w = wbo[pl.ds(pl.multiple_of(h * DM, DM), DM), :]
            ot[:, pl.ds(m * TQ, TQ)] += _dot(w, ctx, _NT)
            yield DM

    def emit_block(m, acc):
        out[pl.ds(m * TQ, TQ), pl.ds(DM, DM)] = acc.astype(bf16).T
        out_copy(m).start()

    def b_outproj_last(m):
        acc = None
        for h in range(H):
            ctx = _unpack(qc[h, pl.ds(m * TQ // 2, TQ // 2), :])
            d = _dot(wbo[pl.ds(h * DM, DM), :], ctx, _NT)
            acc = d if acc is None else acc + d
            yield 2
        emit_block(m, acc)

    def emit_blocks(blocks):
        for m in blocks:
            emit_block(m, ot[:, pl.ds(m * TQ, TQ)])
            yield 1

    def a_absorb(j):
        lane = lax.broadcasted_iota(jnp.int32, (DM, 128), 1)
        tails = []
        for e in range(2):
            wrows = pl.ds(pl.multiple_of((2 * j + e) * (DM // 2), 32), DM // 2)
            wv = _unpack(jnp.concatenate([rawq[0, wrows, :], rawq[1, wrows, :]], axis=1))
            r0 = pl.multiple_of((2 * j + e) * DM, 64)
            wa[j, :, pl.ds(4 * DH + e * DMM, DMM)] = _pack(_dot(wv, wao[pl.ds(r0, DMM), :], _NT))
            yield 3
            rt = pl.multiple_of(r0 + DMM - 64 * e, 64)
            tails.append(_dot(wv, wao[pl.ds(rt, 128), :], _NT))
            yield 1
        wa[j, :, pl.ds(4 * DH + 2 * DMM, 128)] = _pack(jnp.where(lane < 64, tails[0], tails[1]))

    def a_steps(s0, nsteps, state):
        row = lax.broadcasted_iota(jnp.int32, (L, 128), 0)
        col = lax.broadcasted_iota(jnp.int32, (L, 128), 1)
        key = col - jnp.where(col >= 2 * L, 2 * L, jnp.where(col >= L, L, 0))
        mask = (row < MEM) | (row >= key)
        seg_of = [(col >= g * L) & (col < (g + 1) * L) for g in range(3)]

        def pick(xs):
            r = xs[-1]
            for g in range(len(xs) - 2, -1, -1):
                r = jnp.where(col < (g + 1) * L, xs[g], r)
            return r

        def stack(xs):
            pad = jnp.zeros((128 - L * len(xs), xs[0].shape[1]), f32)
            return jnp.concatenate(xs + [pad], axis=0).astype(bf16)

        for ds in range(nsteps):
            r0, p0 = (s0 + ds) * seg, (s0 + ds) * (seg // 2)
            r0, p0 = pl.multiple_of(r0, seg), pl.multiple_of(p0, seg // 2)
            hx = jnp.concatenate([state[0], _unpack(xa[pl.ds(p0, seg // 2), :]).astype(f32)], axis=0)
            qs, ks, zs, ss, ps = {}, {}, {}, {}, {}
            acc = [None]

            def project(j):
                qk = _dot(hx, _unpack(wa[j, :, pl.ds(0, 4 * DH)]))
                for e in range(2):
                    qs[2 * j + e] = qk[:, 2 * e * DH:(2 * e + 1) * DH]
                    ks[2 * j + e] = qk[:, (2 * e + 1) * DH:(2 * e + 2) * DH]

            def project_z(j):
                z = _dot(hx, _unpack(wa[j, :, pl.ds(4 * DH, 2 * DMM + 128)]))
                for e in range(2):
                    tail = jnp.where((col < 64) if e == 0 else (col >= 64), z[:, 2 * DMM:], 0.0)
                    zs[2 * j + e] = jnp.concatenate([z[:, e * DMM:(e + 1) * DMM], tail], axis=1)

            def score(g):
                hs = GROUPS[g]
                r = _dot(jnp.concatenate([qs[h] for h in hs], axis=0), stack([ks[h] for h in hs]), _NT)
                ss[g] = pick([r[n * L:(n + 1) * L] for n in range(len(hs))])

            def soft(g):
                n = len(GROUPS[g])
                s = jnp.where(mask, ss[g] * SCALE, NEG)
                m = pick([jnp.max(jnp.where(seg_of[i], s, -jnp.inf), axis=1, keepdims=True) for i in range(n)])
                p = jnp.where(col < n * L, jnp.exp(s - m), 0.0)
                l = pick([jnp.sum(jnp.where(seg_of[i], p, 0.0), axis=1, keepdims=True) for i in range(n)])
                ps[g] = p / l

            def mix(g):
                d = _dot(ps[g], stack([zs[h] for h in GROUPS[g]]))
                acc[0] = d if acc[0] is None else acc[0] + d

            ops = {"p": project, "z": project_z, "s": score, "f": soft, "m": mix}
            for stage, cst in ASCHED:
                for op in stage.split():
                    ops[op[0]](int(op[1]))
                if stage is ASCHED[-1][0]:
                    t = acc[0][:, DMM:]
                    o = jnp.concatenate([acc[0][:, :DMM], (t + pltpu.roll(t, 64, 1))[:, :64]], axis=1)
                    out[pl.ds(r0, seg), pl.ds(0, DM)] = o[MEM:].astype(bf16)
                    state[0] = o[:MEM].astype(bf16).astype(f32)
                yield cst

    ATT_COST = 17408
    per_head = S // seg // H
    assert per_head * H * seg == S and 3 * L <= 128

    start(cp_bq + xb_copy(0) + xb_copy(1) + cp_bk + cp_bv + cp_av + cp_a + cp_last)
    ot[...] = jnp.zeros_like(ot)
    wait(cp_bq)
    deinterleave(rawq, wbq, lambda h, e: (h, 0, 128 * e), DM)
    n_t = S // 256 // QN

    def xb_body(m, _):
        _merge((transpose_x(xtb, xb, m), 1))
        return 0
    wait(xb_copy(0))
    lax.fori_loop(0, n_t, xb_body, 0)

    nq, n_kv, n_a = H * QN, DC // CH, DM // CH
    n0 = nq - n_kv - n_a

    def q_body(u, _):
        _merge((b_qproj(u), 1))
        return 0
    lax.fori_loop(0, n0, q_body, 0)
    wait(xb_copy(1))
    lax.fori_loop(n_t, QN * n_t, xb_body, 0)
    wait(cp_bk)

    def q2_body(t, _):
        pl.when(t == n_kv // 2)(lambda: wait(cp_bv))
        w, t2 = t // (n_kv // 2), t % (n_kv // 2)
        de = _chain(*[_deinterleave_chunk(rawkv.at[w], wbkv, lambda h, e: (w * H + h, 0, 128 * e), 2 * t2 + i)
                      for i in range(2)])
        _merge((b_qproj(n0 + t), 4096 // QN), (de, 32))
        return 0
    lax.fori_loop(0, n_kv, q2_body, 0)
    wait(cp_av)

    def q3_body(t, _):
        _merge((b_qproj(nq - n_a + t), 4096 // QN),
               (_deinterleave_chunk(raw2, rawq, lambda h, e: (e, h * (DM // 2), 0), t), 16))
        return 0
    lax.fori_loop(0, n_a, q3_body, 0)
    wait(cp_a)

    def absorb_body(j, _):
        t = jnp.minimum(j, n_a - 1)
        de = _chain(*[_deinterleave_chunk(raw, wa, lambda h, e, l=l: (h // 2, 0, (h % 2) * 2 * DH + l + 128 * e), t)
                      for raw, l in ((raw0, 0), (raw1, DH))])
        _merge((a_absorb(j), 8), (de, 32), (transpose_x(xta, xa, j), 1))
        return 0
    lax.fori_loop(0, H // 2, absorb_body, 0)
    wait(cp_last)

    nb = S // TQ
    a_cost = sum(c_ for _, c_ in ASCHED) * ALEAD

    def head_body(h, mem):
        def kv_body(t, mem):
            state = [mem]
            _merge((a_steps(h * per_head + t, 1, state), a_cost),
                   (_chain(*[b_kvblock(h, t * (nb // 2) + m) for m in range(nb // 2)]), nb // 2 * 2048))
            return state[0]
        state = [lax.fori_loop(0, 2, kv_body, mem)]
        fill = {nb: (b_outproj_acc(h, QORDER[:OSPLIT]), OSPLIT * DM),
                nb + 1: (b_outproj_acc(h, QORDER[OSPLIT:-1]), (nb - 1 - OSPLIT) * DM)}
        _merge((a_steps(h * per_head + 2, per_head - 2, state), (per_head - 2) * a_cost),
               (b_attn(h, fill), ATT_COST + (nb - 1) * DM))
        pl.when(h > 0)(lambda: out_copy_a(h - 1).wait())
        out_copy_a(h).start()
        return state[0]
    lax.fori_loop(0, H, head_body, mem0[...].astype(f32))

    _merge((emit_blocks(QORDER[:-1]), 3 * (nb - 1)), (b_outproj_last(QORDER[-1]), 3 * H))
    wait([out_copy(m) for m in range(S // TQ)] + [out_copy_a(H - 1)])


@functools.partial(jax.jit, static_argnames=("A_seg_len",))
def pallas_concat_heads__memory_aug_recurrent_mem_tr__compressed_kv_cla__prompt_kernel(
    A_x, A_mem0, A_Wq, A_Wk, A_Wv, A_Wo, A_seg_len,
    B_x, B_c_kv, B_w_q, B_w_uk, B_w_uv, B_w_o,
):
    args = (
        A_x.reshape(S, DM).T, A_mem0.reshape(MEM, DM),
        A_Wq.reshape(DM * H, DH), A_Wk.reshape(DM * H, DH), A_Wv.reshape(DM * H, DH),
        A_Wo.transpose(0, 2, 1).reshape(H * DM, DH),
        B_x.reshape(S, DM).T, B_c_kv.reshape(S, DC),
        B_w_q.reshape(DM * H, DH), B_w_uk.reshape(DC * H, DH), B_w_uv.reshape(DC * H, DH),
        B_w_o.transpose(0, 2, 1).reshape(H * DM, DH),
    )
    scratch = [
        pltpu.VMEM((DM, S), bf16),
        pltpu.VMEM((DM, S), bf16),
        pltpu.VMEM((S // 2, DM), u32),
        pltpu.VMEM((S // 2, DM), u32),
        pltpu.VMEM((MEM, DM), bf16),
        pltpu.VMEM((H * DM, DH), bf16),
        pltpu.VMEM((S, DC), bf16),
        pltpu.VMEM((H * DM, DH), bf16),
        pltpu.VMEM((2, DM * 8, 128), u32),
        pltpu.VMEM((2, 2, DC * 8, 128), u32),
        pltpu.VMEM((2, DM * 8, 128), u32),
        pltpu.VMEM((2, DM * 8, 128), u32),
        pltpu.VMEM((2, DM * 8, 128), u32),
        pltpu.VMEM((H // 2, DM // 2, 4 * DH + 2 * DMM + 128), u32),
        pltpu.VMEM((H, DM // 2, DH), u32),
        pltpu.VMEM((2 * H, DC // 2, DH), u32),
        pltpu.VMEM((H, S // 2, DH), u32),
        pltpu.VMEM((S // 2, 2 * DH), u32),
        pltpu.VMEM((DM, S), f32),
        pltpu.VMEM((S, 2 * DM), bf16),
        pltpu.SemaphoreType.DMA((20 + S // TQ,)),
    ]
    res = pl.pallas_call(
        functools.partial(_kernel, seg=int(A_seg_len)),
        in_specs=[pl.BlockSpec(memory_space=pl.ANY)] * len(args),
        out_specs=pl.BlockSpec(memory_space=pl.ANY),
        out_shape=jax.ShapeDtypeStruct((S, 2 * DM), bf16),
        scratch_shapes=scratch,
        compiler_params=pltpu.CompilerParams(vmem_limit_bytes=120 << 20),
    )(*args)
    return res.reshape(1, S, 2 * DM)
```

```python
import functools

import jax
import jax.numpy as jnp
from jax import lax
import jax.experimental.pallas as pl
import jax.experimental.pallas.tpu as pltpu

S = 2048
DM = 448
H = 16
DH = 256
DC = 1024
MEM = 8
TQ = 256
HB = 128
QORDER = (1, 2, 3, 7, 6, 5, 4, 0)
SL1 = 2.1
SL2 = 1.4
OSPLIT = 3
RG = 32
DMM = 384
GROUPS = ((0, 1, 2), (3, 4, 5), (6, 7, 8), (9, 10, 11), (12, 13), (14, 15))
ASCHED = (("p0", 320), ("p1", 320), ("p2 s0", 380), ("p3 s1 f0", 380), ("p4 f1", 320), ("p5 s2", 380), ("p6 s3 f2", 380), ("p7 s4 f3", 360), ("z0 s5 f4", 320), ("z1 f5", 280), ("z2 m0", 320), ("z3 m1", 320), ("z4", 280), ("z5 m2", 320), ("z6 m3", 320), ("z7 m4", 320), ("", 200), ("m5", 300))
ALEAD = 1.1
QN = 2
CH = 64
NEG = -1000000000.0
SCALE = DH ** -0.5

_NN = (((1,), (0,)), ((), ()))
_NT = (((1,), (1,)), ((), ()))
bf16, f32, u32 = jnp.bfloat16, jnp.float32, jnp.uint32


def _dot(a, b, dims=_NN):
    return lax.dot_general(a, b, dims, preferred_element_type=f32)


def _pack(x):
    return pltpu.bitcast(x.astype(bf16), u32)


def _unpack(x):
    return pltpu.bitcast(x, bf16)


def _deinterleave_chunk(raw, dst, place, t):
    r0 = t * (CH // 2)
    s0 = t * (CH * 8)
    if not isinstance(t, int):
        r0, s0 = pl.multiple_of(r0, CH // 2), pl.multiple_of(s0, CH * 8)
    for half in range(2):
        src = raw.at[half, pl.ds(s0, CH * 8), :]
        for j in range(8):
            xe = src[pl.ds(j, CH // 2, stride=16), :]
            xo = src[pl.ds(8 + j, CH // 2, stride=16), :]
            vals = ((xe & u32(0xFFFF)) | (xo << 16), (xe >> 16) | (xo & u32(0xFFFF0000)))
            for e in range(2):
                i, r, l = place(2 * j + e, half)
                dst[i, pl.ds(r + r0, CH // 2), pl.ds(l, 128)] = vals[e]
            yield 1


def _chain(*gens):
    for g in gens:
        yield from g


def _zip(main, total, side, count):
    done, n = 0.0, 0
    for cst in main:
        done += cst
        while n < count and n < done / total * count:
            next(side)
            n += 1
        yield cst
    for _ in side:
        pass


def _merge(*streams):
    gens = [g for g, _ in streams]
    totals = [float(t) for _, t in streams]
    done = [0.0] * len(gens)
    live = list(range(len(gens)))
    while live:
        i = min(live, key=lambda n: done[n] / totals[n])
        try:
            done[i] += next(gens[i])
        except StopIteration:
            live.remove(i)


def _kernel(xa_hbm, mem_hbm, aq_hbm, ak_hbm, av_hbm, ao_hbm,
            xb_hbm, c_hbm, bq_hbm, bk_hbm, bv_hbm, bo_hbm,
            o_hbm,
            xta, xtb, xa, xb, mem0, wao, c, wbo, rawq, rawkv, raw0, raw1, raw2,
            wa, wz, wbq, wbkv, qc, kv, ot, out, sems, *, seg):
    L = MEM + seg

    def raw_copies(hbm, raw, s0):
        u = hbm.bitcast(u32)
        return [pltpu.make_async_copy(u.at[:, pl.ds(128 * i, 128)], raw.at[i], sems.at[s0 + i])
                for i in range(2)]

    half = S // QN

    def xb_copy(i):
        cols = pl.ds(i * half, half)
        return [pltpu.make_async_copy(xb_hbm.at[:, cols], xtb.at[:, cols], sems.at[i])]

    cp_bq = raw_copies(bq_hbm, rawq, 2)
    cp_bk = raw_copies(bk_hbm, rawkv.at[0], 4)
    cp_bv = raw_copies(bv_hbm, rawkv.at[1], 6)
    cp_av = raw_copies(av_hbm, raw2, 8)
    cp_a = ([pltpu.make_async_copy(ao_hbm, wao, sems.at[10]),
             pltpu.make_async_copy(xa_hbm, xta, sems.at[11])]
            + raw_copies(aq_hbm, raw0, 12) + raw_copies(ak_hbm, raw1, 14))
    cp_last = [pltpu.make_async_copy(mem_hbm, mem0, sems.at[16]),
               pltpu.make_async_copy(c_hbm, c, sems.at[17]),
               pltpu.make_async_copy(bo_hbm, wbo, sems.at[18])]

    def start(cps):
        for cp in cps:
            cp.start()

    def wait(cps):
        for cp in cps:
            cp.wait()

    def transpose_x(xt, xs, m):
        r = pl.multiple_of(m * 128, 128)
        xs[pl.ds(r, 128), :] = pltpu.bitcast(xt[:, pl.ds(pl.multiple_of(2 * r, 256), 256)].T, u32)
        yield 1

    def deinterleave(raw, dst, place, rows):
        def body(t, _):
            _merge((_deinterleave_chunk(raw, dst, place, t), 1))
            return 0
        lax.fori_loop(0, rows // CH, body, 0)

    def b_qproj(u):
        h, m0 = u % H, (u // H) * (S // QN // 2)
        w = _unpack(wbq[h])
        for m in range(S // QN // 256):
            rows = pl.ds(pl.multiple_of(m0 + m * 128, 128), 128)
            qc[h, rows, :] = _pack(_dot(_unpack(xb[rows, :]), w) * SCALE)
            yield 512

    def b_kvblock(h, m):
        r = m * 128
        if not isinstance(m, int):
            r = pl.multiple_of(r, 128)
        for l0 in (0, DH):
            acc = None
            for k0 in range(0, DC, 512):
                d = _dot(c[pl.ds(2 * r, 256), pl.ds(k0, 512)],
                         _unpack(wbkv[(l0 // DH) * H + h, pl.ds(k0 // 2, 256), :]))
                acc = d if acc is None else acc + d
                if k0 + 512 == DC:
                    kv[pl.ds(r, 128), pl.ds(l0, DH)] = _pack(acc)
                yield 512

    def b_attn(h, fill):
        row = lax.broadcasted_iota(jnp.int32, (HB, HB), 0)
        col = lax.broadcasted_iota(jnp.int32, (HB, HB), 1)
        tri = col <= row
        conv = lambda r0, nr, l0: _unpack(kv[pl.ds(r0 // 2, nr // 2), pl.ds(l0, DH)])

        def blocks(i):
            return [(j * TQ, TQ) for j in range(i)] + [(i * TQ, HB)]

        def scores(i, st):
            q = _unpack(qc[h, pl.ds(i * TQ // 2, TQ // 2), :])
            st["s"] = []
            for k0, nk in blocks(i):
                st["s"].append(_dot(q, conv(k0, nk, 0), _NT))
                yield nk
            st["sb"] = _dot(q[HB:], conv(i * TQ + HB, HB, 0), _NT)
            yield HB // 2

        def softmax(i, st):
            st["p"], st["pb"], st["l"] = [], [], []
            for r in range(0, TQ, RG):
                parts = [x[r:r + RG] for x in st["s"]]
                if r < HB:
                    parts[-1] = jnp.where(tri[r:r + RG], parts[-1], NEG)
                else:
                    parts.append(jnp.where(tri[r - HB:r - HB + RG], st["sb"][r - HB:r - HB + RG], NEG))
                s = jnp.concatenate(parts, axis=1)
                p = jnp.exp(s - jnp.max(s, axis=1, keepdims=True))
                st["l"].append(jnp.sum(p, axis=1, keepdims=True))
                p = p.astype(bf16)
                n = i * TQ + HB
                st["p"].append(p[:, :n])
                if r >= HB:
                    st["pb"].append(p[:, n:])
                yield 0

        def values(i, st):
            o = None
            for k0, nk in blocks(i):
                d = _dot(jnp.concatenate([x[:, k0:k0 + nk] for x in st["p"]], axis=0), conv(k0, nk, DH))
                o = d if o is None else o + d
                yield nk
            ob = _dot(jnp.concatenate(st["pb"], axis=0), conv(i * TQ + HB, HB, DH))
            o = jnp.concatenate([o[:HB], o[HB:] + ob], axis=0) / jnp.concatenate(st["l"], axis=0)
            qc[h, pl.ds(i * TQ // 2, TQ // 2), :] = _pack(o)
            yield HB // 2

        cost = lambda i: i * TQ + HB + HB // 2
        sts = [{} for _ in QORDER]
        for t in range(len(QORDER) + 2):
            mxu, tot = [], 0
            if t in fill:
                mxu.append(fill[t][0])
                tot += fill[t][1]
            if t >= 2:
                mxu.append(values(QORDER[t - 2], sts[t - 2]))
                tot += cost(QORDER[t - 2])
            if t < len(QORDER):
                mxu.append(scores(QORDER[t], sts[t]))
                tot += cost(QORDER[t])
            if 1 <= t <= len(QORDER):
                yield from _zip(_chain(*mxu), tot, softmax(QORDER[t - 1], sts[t - 1]), TQ // RG)
            else:
                yield from _chain(*mxu)

    def out_copy(m):
        rows, lanes = pl.ds(m * TQ, TQ), pl.ds(DMM, 2 * DM - DMM)
        return pltpu.make_async_copy(out.at[rows, lanes], o_hbm.at[rows, lanes], sems.at[19 + m])

    def out_copy_a(h):
        n = S // H
        rows, lanes = pl.ds(pl.multiple_of(h * n, n), n), pl.ds(0, DMM)
        return pltpu.make_async_copy(out.at[rows, lanes], o_hbm.at[rows, lanes], sems.at[19 + S // TQ])

    def b_outproj_acc(h, blocks):
        for m in blocks:
            ctx = _unpack(qc[h, pl.ds(m * TQ // 2, TQ // 2), :])
            w = wbo[pl.ds(pl.multiple_of(h * DM, DM), DM), :]
            ot[:, pl.ds(m * TQ, TQ)] += _dot(w, ctx, _NT)
            yield DM

    def emit_block(m, acc):
        out[pl.ds(m * TQ, TQ), pl.ds(DM, DM)] = acc.astype(bf16).T
        out_copy(m).start()

    def b_outproj_last(m):
        acc = None
        for h in range(H):
            ctx = _unpack(qc[h, pl.ds(m * TQ // 2, TQ // 2), :])
            d = _dot(wbo[pl.ds(h * DM, DM), :], ctx, _NT)
            acc = d if acc is None else acc + d
            yield 2
        emit_block(m, acc)

    def emit_blocks(blocks):
        for m in blocks:
            emit_block(m, ot[:, pl.ds(m * TQ, TQ)])
            yield 1

    def a_absorb(j):
        lane = lax.broadcasted_iota(jnp.int32, (DM, 128), 1)
        tails = []
        for e in range(2):
            wrows = pl.ds(pl.multiple_of((2 * j + e) * (DM // 2), 32), DM // 2)
            wv = _unpack(jnp.concatenate([rawq[0, wrows, :], rawq[1, wrows, :]], axis=1))
            r0 = pl.multiple_of((2 * j + e) * DM, 64)
            rt = pl.multiple_of(r0 + DMM - 64 * e, 64)
            wo = jnp.concatenate([wao[pl.ds(r0, DMM), :], wao[pl.ds(rt, 128), :]], axis=0)
            d = _dot(wv, wo, _NT)
            wz[j, :, pl.ds(e * DMM, DMM)] = _pack(d[:, :DMM])
            tails.append(d[:, DMM:])
            yield 4
        wz[j, :, pl.ds(2 * DMM, 128)] = _pack(jnp.where(lane < 64, tails[0], tails[1]))

    def a_steps(s0, nsteps, state):
        row = lax.broadcasted_iota(jnp.int32, (L, 128), 0)
        col = lax.broadcasted_iota(jnp.int32, (L, 128), 1)
        key = col - jnp.where(col >= 2 * L, 2 * L, jnp.where(col >= L, L, 0))
        mask = (row < MEM) | (row >= key)
        seg_of = [(col >= g * L) & (col < (g + 1) * L) for g in range(3)]

        def pick(xs):
            r = xs[-1]
            for g in range(len(xs) - 2, -1, -1):
                r = jnp.where(col < (g + 1) * L, xs[g], r)
            return r

        def stack(xs):
            pad = jnp.zeros((128 - L * len(xs), xs[0].shape[1]), f32)
            return jnp.concatenate(xs + [pad], axis=0).astype(bf16)

        for ds in range(nsteps):
            r0, p0 = (s0 + ds) * seg, (s0 + ds) * (seg // 2)
            r0, p0 = pl.multiple_of(r0, seg), pl.multiple_of(p0, seg // 2)
            hx = jnp.concatenate([state[0], _unpack(xa[pl.ds(p0, seg // 2), :]).astype(f32)], axis=0)
            qs, ks, zs, ss, ps = {}, {}, {}, {}, {}
            acc = [None]

            def project(j):
                qk = _dot(hx, _unpack(wa[j]))
                for e in range(2):
                    qs[2 * j + e] = qk[:, 2 * e * DH:(2 * e + 1) * DH]
                    ks[2 * j + e] = qk[:, (2 * e + 1) * DH:(2 * e + 2) * DH]

            def project_z(j):
                z = _dot(hx, _unpack(wz[j]))
                for e in range(2):
                    tail = jnp.where((col < 64) if e == 0 else (col >= 64), z[:, 2 * DMM:], 0.0)
                    zs[2 * j + e] = jnp.concatenate([z[:, e * DMM:(e + 1) * DMM], tail], axis=1)

            def score(g):
                hs = GROUPS[g]
                r = _dot(jnp.concatenate([qs[h] for h in hs], axis=0), stack([ks[h] for h in hs]), _NT)
                ss[g] = pick([r[n * L:(n + 1) * L] for n in range(len(hs))])

            def soft(g):
                n = len(GROUPS[g])
                s = jnp.where(mask, ss[g] * SCALE, NEG)
                m = pick([jnp.max(jnp.where(seg_of[i], s, -jnp.inf), axis=1, keepdims=True) for i in range(n)])
                p = jnp.where(col < n * L, jnp.exp(s - m), 0.0)
                l = pick([jnp.sum(jnp.where(seg_of[i], p, 0.0), axis=1, keepdims=True) for i in range(n)])
                ps[g] = p / l

            def mix(g):
                d = _dot(ps[g], stack([zs[h] for h in GROUPS[g]]))
                acc[0] = d if acc[0] is None else acc[0] + d

            ops = {"p": project, "z": project_z, "s": score, "f": soft, "m": mix}
            for stage, cst in ASCHED:
                for op in stage.split():
                    ops[op[0]](int(op[1]))
                if stage is ASCHED[-1][0]:
                    t = acc[0][:, DMM:]
                    o = jnp.concatenate([acc[0][:, :DMM], (t + pltpu.roll(t, 64, 1))[:, :64]], axis=1)
                    out[pl.ds(r0, seg), pl.ds(0, DM)] = o[MEM:].astype(bf16)
                    state[0] = o[:MEM].astype(bf16).astype(f32)
                yield cst

    ATT_COST = 17408
    per_head = S // seg // H
    assert per_head * H * seg == S and 3 * L <= 128

    start(cp_bq + xb_copy(0) + xb_copy(1) + cp_bk + cp_bv + cp_av + cp_a + cp_last)
    ot[...] = jnp.zeros_like(ot)
    wait(cp_bq)
    deinterleave(rawq, wbq, lambda h, e: (h, 0, 128 * e), DM)
    n_t = S // 256 // QN

    def xb_body(m, _):
        _merge((transpose_x(xtb, xb, m), 1))
        return 0
    wait(xb_copy(0))
    lax.fori_loop(0, n_t, xb_body, 0)

    nq, n_kv, n_a = H * QN, DC // CH, DM // CH
    n0 = nq - n_kv - n_a

    def q_body(u, _):
        _merge((b_qproj(u), 1))
        return 0
    lax.fori_loop(0, n0, q_body, 0)
    wait(xb_copy(1))
    lax.fori_loop(n_t, QN * n_t, xb_body, 0)
    wait(cp_bk)

    def q2_body(t, _):
        pl.when(t == n_kv // 2)(lambda: wait(cp_bv))
        w, t2 = t // (n_kv // 2), t % (n_kv // 2)
        de = _chain(*[_deinterleave_chunk(rawkv.at[w], wbkv, lambda h, e: (w * H + h, 0, 128 * e), 2 * t2 + i)
                      for i in range(2)])
        _merge((de, 32 * SL2), (b_qproj(n0 + t), 4096 // QN))
        return 0
    lax.fori_loop(0, n_kv, q2_body, 0)
    wait(cp_av)

    def q3_body(t, _):
        _merge((b_qproj(nq - n_a + t), 4096 // QN),
               (_deinterleave_chunk(raw2, rawq, lambda h, e: (e, h * (DM // 2), 0), t), 16 * SL2))
        return 0
    lax.fori_loop(0, n_a, q3_body, 0)
    wait(cp_a)

    def absorb_body(j, _):
        t = jnp.minimum(j, n_a - 1)
        de = _chain(*[_deinterleave_chunk(raw, wa, lambda h, e, l=l: (h // 2, 0, (h % 2) * 2 * DH + l + 128 * e), t)
                      for raw, l in ((raw0, 0), (raw1, DH))])
        _merge((transpose_x(xta, xa, j), 1), (de, 32 * SL1), (a_absorb(j), 8))
        return 0
    lax.fori_loop(0, H // 2, absorb_body, 0)
    wait(cp_last)

    nb = S // TQ
    a_cost = sum(c_ for _, c_ in ASCHED) * ALEAD

    def head_body(h, mem):
        def kv_body(t, mem):
            state = [mem]
            _merge((a_steps(h * per_head + t, 1, state), a_cost),
                   (_chain(*[b_kvblock(h, t * (nb // 2) + m) for m in range(nb // 2)]), nb // 2 * 2048))
            return state[0]
        state = [lax.fori_loop(0, 2, kv_body, mem)]
        fill = {nb: (b_outproj_acc(h, QORDER[:OSPLIT]), OSPLIT * DM),
                nb + 1: (b_outproj_acc(h, QORDER[OSPLIT:-1]), (nb - 1 - OSPLIT) * DM)}
        _merge((a_steps(h * per_head + 2, per_head - 2, state), (per_head - 2) * a_cost),
               (b_attn(h, fill), ATT_COST + (nb - 1) * DM))
        pl.when(h > 0)(lambda: out_copy_a(h - 1).wait())
        out_copy_a(h).start()
        return state[0]
    lax.fori_loop(0, H, head_body, mem0[...].astype(f32))

    _merge((emit_blocks(QORDER[:-1]), 3 * (nb - 1)), (b_outproj_last(QORDER[-1]), 3 * H))
    wait([out_copy(m) for m in range(S // TQ)] + [out_copy_a(H - 1)])


@functools.partial(jax.jit, static_argnames=("A_seg_len",))
def pallas_concat_heads__memory_aug_recurrent_mem_tr__compressed_kv_cla__prompt_kernel(
    A_x, A_mem0, A_Wq, A_Wk, A_Wv, A_Wo, A_seg_len,
    B_x, B_c_kv, B_w_q, B_w_uk, B_w_uv, B_w_o,
):
    args = (
        A_x.reshape(S, DM).T, A_mem0.reshape(MEM, DM),
        A_Wq.reshape(DM * H, DH), A_Wk.reshape(DM * H, DH), A_Wv.reshape(DM * H, DH),
        A_Wo.transpose(0, 2, 1).reshape(H * DM, DH),
        B_x.reshape(S, DM).T, B_c_kv.reshape(S, DC),
        B_w_q.reshape(DM * H, DH), B_w_uk.reshape(DC * H, DH), B_w_uv.reshape(DC * H, DH),
        B_w_o.transpose(0, 2, 1).reshape(H * DM, DH),
    )
    scratch = [
        pltpu.VMEM((DM, S), bf16),
        pltpu.VMEM((DM, S), bf16),
        pltpu.VMEM((S // 2, DM), u32),
        pltpu.VMEM((S // 2, DM), u32),
        pltpu.VMEM((MEM, DM), bf16),
        pltpu.VMEM((H * DM, DH), bf16),
        pltpu.VMEM((S, DC), bf16),
        pltpu.VMEM((H * DM, DH), bf16),
        pltpu.VMEM((2, DM * 8, 128), u32),
        pltpu.VMEM((2, 2, DC * 8, 128), u32),
        pltpu.VMEM((2, DM * 8, 128), u32),
        pltpu.VMEM((2, DM * 8, 128), u32),
        pltpu.VMEM((2, DM * 8, 128), u32),
        pltpu.VMEM((H // 2, DM // 2, 4 * DH), u32),
        pltpu.VMEM((H // 2, DM // 2, 2 * DMM + 128), u32),
        pltpu.VMEM((H, DM // 2, DH), u32),
        pltpu.VMEM((2 * H, DC // 2, DH), u32),
        pltpu.VMEM((H, S // 2, DH), u32),
        pltpu.VMEM((S // 2, 2 * DH), u32),
        pltpu.VMEM((DM, S), f32),
        pltpu.VMEM((S, 2 * DM), bf16),
        pltpu.SemaphoreType.DMA((20 + S // TQ,)),
    ]
    res = pl.pallas_call(
        functools.partial(_kernel, seg=int(A_seg_len)),
        in_specs=[pl.BlockSpec(memory_space=pl.ANY)] * len(args),
        out_specs=pl.BlockSpec(memory_space=pl.ANY),
        out_shape=jax.ShapeDtypeStruct((S, 2 * DM), bf16),
        scratch_shapes=scratch,
        compiler_params=pltpu.CompilerParams(vmem_limit_bytes=120 << 20),
    )(*args)
    return res.reshape(1, S, 2 * DM)
```

```python
import functools

import jax
import jax.numpy as jnp
from jax import lax
import jax.experimental.pallas as pl
import jax.experimental.pallas.tpu as pltpu

S = 2048
DM = 448
H = 16
DH = 256
DC = 1024
MEM = 8
TQ = 256
HB = 128
QORDER = (1, 2, 3, 7, 6, 5, 4, 0)
SL1 = 2.1
SL2 = 1.4
OSPLIT = 3
RG = 32
DMM = 384
GROUPS = ((1, 2, 3), (4, 5, 6), (7, 8, 9), (10, 11, 12), (13, 14, 15), (0,))
ASCHED = (("p0", 320), ("p1 s5", 340), ("p2 s0", 380), ("p3 f5", 320), ("p4 s1 f0", 380), ("p5 s2", 380),
          ("p6 f1", 320), ("p7 s3 f2", 380), ("z0 s4", 340), ("z1 f3", 280), ("z2 f4 m0", 320), ("z3", 280),
          ("z4 m1", 320), ("z5 m2", 320), ("z6", 280), ("z7 m3", 320), ("", 200), ("m4", 300))
ALEAD = 1.1
QN = 2
CH = 64
NEG = -1000000000.0
SCALE = DH ** -0.5

_NN = (((1,), (0,)), ((), ()))
_NT = (((1,), (1,)), ((), ()))
bf16, f32, u32 = jnp.bfloat16, jnp.float32, jnp.uint32


def _dot(a, b, dims=_NN):
    return lax.dot_general(a, b, dims, preferred_element_type=f32)


def _pack(x):
    return pltpu.bitcast(x.astype(bf16), u32)


def _unpack(x):
    return pltpu.bitcast(x, bf16)


def _deinterleave_chunk(raw, dst, place, t):
    r0 = t * (CH // 2)
    s0 = t * (CH * 8)
    if not isinstance(t, int):
        r0, s0 = pl.multiple_of(r0, CH // 2), pl.multiple_of(s0, CH * 8)
    for half in range(2):
        src = raw.at[half, pl.ds(s0, CH * 8), :]
        for j in range(8):
            xe = src[pl.ds(j, CH // 2, stride=16), :]
            xo = src[pl.ds(8 + j, CH // 2, stride=16), :]
            vals = ((xe & u32(0xFFFF)) | (xo << 16), (xe >> 16) | (xo & u32(0xFFFF0000)))
            for e in range(2):
                i, r, l = place(2 * j + e, half)
                dst[i, pl.ds(r + r0, CH // 2), pl.ds(l, 128)] = vals[e]
            yield 1


def _chain(*gens):
    for g in gens:
        yield from g


def _zip(main, total, side, count):
    done, n = 0.0, 0
    for cst in main:
        done += cst
        while n < count and n < done / total * count:
            next(side)
            n += 1
        yield cst
    for _ in side:
        pass


def _merge(*streams):
    gens = [g for g, _ in streams]
    totals = [float(t) for _, t in streams]
    done = [0.0] * len(gens)
    live = list(range(len(gens)))
    while live:
        i = min(live, key=lambda n: done[n] / totals[n])
        try:
            done[i] += next(gens[i])
        except StopIteration:
            live.remove(i)


def _kernel(xa_hbm, mem_hbm, aq_hbm, ak_hbm, av_hbm, ao_hbm,
            xb_hbm, c_hbm, bq_hbm, bk_hbm, bv_hbm, bo_hbm,
            o_hbm,
            xta, xtb, xa, xb, mem0, wao, c, wbo, rawq, rawkv, raw0, raw1, raw2,
            wa, wz, wbq, wbkv, qc, kv, ot, out, sems, *, seg):
    L = MEM + seg

    def raw_copies(hbm, raw, s0):
        u = hbm.bitcast(u32)
        return [pltpu.make_async_copy(u.at[:, pl.ds(128 * i, 128)], raw.at[i], sems.at[s0 + i])
                for i in range(2)]

    half = S // QN

    def xb_copy(i):
        cols = pl.ds(i * half, half)
        return [pltpu.make_async_copy(xb_hbm.at[:, cols], xtb.at[:, cols], sems.at[i])]

    cp_bq = raw_copies(bq_hbm, rawq, 2)
    cp_bk = raw_copies(bk_hbm, rawkv.at[0], 4)
    cp_bv = raw_copies(bv_hbm, rawkv.at[1], 6)
    cp_av = raw_copies(av_hbm, raw2, 8)
    cp_a = ([pltpu.make_async_copy(ao_hbm, wao, sems.at[10]),
             pltpu.make_async_copy(xa_hbm, xta, sems.at[11])]
            + raw_copies(aq_hbm, raw0, 12) + raw_copies(ak_hbm, raw1, 14))
    cp_last = [pltpu.make_async_copy(mem_hbm, mem0, sems.at[16]),
               pltpu.make_async_copy(c_hbm, c, sems.at[17]),
               pltpu.make_async_copy(bo_hbm, wbo, sems.at[18])]

    def start(cps):
        for cp in cps:
            cp.start()

    def wait(cps):
        for cp in cps:
            cp.wait()

    def transpose_x(xt, xs, m):
        r = pl.multiple_of(m * 128, 128)
        xs[pl.ds(r, 128), :] = pltpu.bitcast(xt[:, pl.ds(pl.multiple_of(2 * r, 256), 256)].T, u32)
        yield 1

    def deinterleave(raw, dst, place, rows):
        def body(t, _):
            _merge((_deinterleave_chunk(raw, dst, place, t), 1))
            return 0
        lax.fori_loop(0, rows // CH, body, 0)

    def b_qproj(u):
        h, m0 = u % H, (u // H) * (S // QN // 2)
        w = _unpack(wbq[h])
        for m in range(S // QN // 256):
            rows = pl.ds(pl.multiple_of(m0 + m * 128, 128), 128)
            qc[h, rows, :] = _pack(_dot(_unpack(xb[rows, :]), w) * SCALE)
            yield 512

    def b_kvblock(h, m):
        r = m * 128
        if not isinstance(m, int):
            r = pl.multiple_of(r, 128)
        for l0 in (0, DH):
            acc = None
            for k0 in range(0, DC, 512):
                d = _dot(c[pl.ds(2 * r, 256), pl.ds(k0, 512)],
                         _unpack(wbkv[(l0 // DH) * H + h, pl.ds(k0 // 2, 256), :]))
                acc = d if acc is None else acc + d
                if k0 + 512 == DC:
                    kv[pl.ds(r, 128), pl.ds(l0, DH)] = _pack(acc)
                yield 512

    def b_attn(h, fill):
        row = lax.broadcasted_iota(jnp.int32, (HB, HB), 0)
        col = lax.broadcasted_iota(jnp.int32, (HB, HB), 1)
        tri = col <= row
        conv = lambda r0, nr, l0: _unpack(kv[pl.ds(r0 // 2, nr // 2), pl.ds(l0, DH)])

        def blocks(i):
            return [(j * TQ, TQ) for j in range(i)] + [(i * TQ, HB)]

        def scores(i, st):
            q = _unpack(qc[h, pl.ds(i * TQ // 2, TQ // 2), :])
            st["s"] = []
            for k0, nk in blocks(i):
                st["s"].append(_dot(q, conv(k0, nk, 0), _NT))
                yield nk
            st["sb"] = _dot(q[HB:], conv(i * TQ + HB, HB, 0), _NT)
            yield HB // 2

        def softmax(i, st):
            st["p"], st["pb"], st["l"] = [], [], []
            for r in range(0, TQ, RG):
                parts = [x[r:r + RG] for x in st["s"]]
                if r < HB:
                    parts[-1] = jnp.where(tri[r:r + RG], parts[-1], NEG)
                else:
                    parts.append(jnp.where(tri[r - HB:r - HB + RG], st["sb"][r - HB:r - HB + RG], NEG))
                s = jnp.concatenate(parts, axis=1)
                p = jnp.exp(s - jnp.max(s, axis=1, keepdims=True))
                st["l"].append(jnp.sum(p, axis=1, keepdims=True))
                p = p.astype(bf16)
                n = i * TQ + HB
                st["p"].append(p[:, :n])
                if r >= HB:
                    st["pb"].append(p[:, n:])
                yield 0

        def values(i, st):
            o = None
            for k0, nk in blocks(i):
                d = _dot(jnp.concatenate([x[:, k0:k0 + nk] for x in st["p"]], axis=0), conv(k0, nk, DH))
                o = d if o is None else o + d
                yield nk
            ob = _dot(jnp.concatenate(st["pb"], axis=0), conv(i * TQ + HB, HB, DH))
            o = jnp.concatenate([o[:HB], o[HB:] + ob], axis=0) / jnp.concatenate(st["l"], axis=0)
            qc[h, pl.ds(i * TQ // 2, TQ // 2), :] = _pack(o)
            yield HB // 2

        cost = lambda i: i * TQ + HB + HB // 2
        sts = [{} for _ in QORDER]
        for t in range(len(QORDER) + 2):
            mxu, tot = [], 0
            if t in fill:
                mxu.append(fill[t][0])
                tot += fill[t][1]
            if t >= 2:
                mxu.append(values(QORDER[t - 2], sts[t - 2]))
                tot += cost(QORDER[t - 2])
            if t < len(QORDER):
                mxu.append(scores(QORDER[t], sts[t]))
                tot += cost(QORDER[t])
            if 1 <= t <= len(QORDER):
                yield from _zip(_chain(*mxu), tot, softmax(QORDER[t - 1], sts[t - 1]), TQ // RG)
            else:
                yield from _chain(*mxu)

    def out_copy(m):
        rows, lanes = pl.ds(m * TQ, TQ), pl.ds(DMM, 2 * DM - DMM)
        return pltpu.make_async_copy(out.at[rows, lanes], o_hbm.at[rows, lanes], sems.at[19 + m])

    def out_copy_a(h):
        n = S // H
        rows, lanes = pl.ds(pl.multiple_of(h * n, n), n), pl.ds(0, DMM)
        return pltpu.make_async_copy(out.at[rows, lanes], o_hbm.at[rows, lanes], sems.at[19 + S // TQ])

    def b_outproj_acc(h, blocks):
        for m in blocks:
            ctx = _unpack(qc[h, pl.ds(m * TQ // 2, TQ // 2), :])
            w = wbo[pl.ds(pl.multiple_of(h * DM, DM), DM), :]
            ot[:, pl.ds(m * TQ, TQ)] += _dot(w, ctx, _NT)
            yield DM

    def emit_block(m, acc):
        out[pl.ds(m * TQ, TQ), pl.ds(DM, DM)] = acc.astype(bf16).T
        out_copy(m).start()

    def b_outproj_last(m):
        acc = None
        for h in range(H):
            ctx = _unpack(qc[h, pl.ds(m * TQ // 2, TQ // 2), :])
            d = _dot(wbo[pl.ds(h * DM, DM), :], ctx, _NT)
            acc = d if acc is None else acc + d
            yield 2
        emit_block(m, acc)

    def emit_blocks(blocks):
        for m in blocks:
            emit_block(m, ot[:, pl.ds(m * TQ, TQ)])
            yield 1

    def a_absorb(j):
        lane = lax.broadcasted_iota(jnp.int32, (DM, 128), 1)
        tails = []
        for e in range(2):
            wrows = pl.ds(pl.multiple_of((2 * j + e) * (DM // 2), 32), DM // 2)
            wv = _unpack(jnp.concatenate([rawq[0, wrows, :], rawq[1, wrows, :]], axis=1))
            r0 = pl.multiple_of((2 * j + e) * DM, 64)
            rt = pl.multiple_of(r0 + DMM - 64 * e, 64)
            wo = jnp.concatenate([wao[pl.ds(r0, DMM), :], wao[pl.ds(rt, 128), :]], axis=0)
            d = _dot(wv, wo, _NT)
            wz[j, :, pl.ds(e * DMM, DMM)] = _pack(d[:, :DMM])
            tails.append(d[:, DMM:])
            yield 4
        wz[j, :, pl.ds(2 * DMM, 128)] = _pack(jnp.where(lane < 64, tails[0], tails[1]))

    def a_steps(s0, nsteps, state):
        row = lax.broadcasted_iota(jnp.int32, (L, 128), 0)
        col = lax.broadcasted_iota(jnp.int32, (L, 128), 1)
        key = col - jnp.where(col >= 2 * L, 2 * L, jnp.where(col >= L, L, 0))
        mask = (row < MEM) | (row >= key)
        spare = 128 - 3 * L
        seg_of = [(col >= g * L) & (col < (g + 1) * L) for g in range(3)]

        def pick(xs):
            r = xs[-1]
            for g in range(len(xs) - 2, -1, -1):
                r = jnp.where(col < (g + 1) * L, xs[g], r)
            return r

        def stack(xs):
            pad = 128 - sum(x.shape[0] for x in xs)
            if pad:
                xs = xs + [jnp.zeros((pad, xs[0].shape[1]), f32)]
            return jnp.concatenate(xs, axis=0).astype(bf16)

        for ds in range(nsteps):
            r0, p0 = (s0 + ds) * seg, (s0 + ds) * (seg // 2)
            r0, p0 = pl.multiple_of(r0, seg), pl.multiple_of(p0, seg // 2)
            hx = jnp.concatenate([state[0], _unpack(xa[pl.ds(p0, seg // 2), :]).astype(f32)], axis=0)
            qs, ks, zs, ss, ps = {}, {}, {}, {}, {}
            acc = [None]

            def project(j):
                qk = _dot(hx, _unpack(wa[j]))
                for e in range(2):
                    qs[2 * j + e] = qk[:, 2 * e * DH:(2 * e + 1) * DH]
                    ks[2 * j + e] = qk[:, (2 * e + 1) * DH:(2 * e + 2) * DH]

            def project_z(j):
                z = _dot(hx, _unpack(wz[j]))
                for e in range(2):
                    tail = jnp.where((col < 64) if e == 0 else (col >= 64), z[:, 2 * DMM:], 0.0)
                    zs[2 * j + e] = jnp.concatenate([z[:, e * DMM:(e + 1) * DMM], tail], axis=1)

            def score(g):
                hs = GROUPS[g]
                r = _dot(jnp.concatenate([qs[h] for h in hs], axis=0), stack([ks[h] for h in hs]), _NT)
                ss[g] = pick([r[n * L:(n + 1) * L] for n in range(len(hs))])

            def soft(g):
                n = len(GROUPS[g])
                s = jnp.where(mask, ss[g] * SCALE, NEG)
                m = pick([jnp.max(jnp.where(seg_of[i], s, -jnp.inf), axis=1, keepdims=True) for i in range(n)])
                p = jnp.where(col < n * L, jnp.exp(s - m), 0.0)
                l = pick([jnp.sum(jnp.where(seg_of[i], p, 0.0), axis=1, keepdims=True) for i in range(n)])
                ps[g] = p / l

            def mix(g):
                last = len(GROUPS) - 1
                p = jnp.where(col < 3 * L, ps[g], pltpu.roll(ps[last], 3 * L - spare * g, 1))
                extra = zs[GROUPS[last][0]][spare * g:spare * (g + 1)]
                d = _dot(p, stack([zs[h] for h in GROUPS[g]] + [extra]))
                acc[0] = d if acc[0] is None else acc[0] + d

            ops = {"p": project, "z": project_z, "s": score, "f": soft, "m": mix}
            for stage, cst in ASCHED:
                for op in stage.split():
                    ops[op[0]](int(op[1]))
                if stage is ASCHED[-1][0]:
                    t = acc[0][:, DMM:]
                    o = jnp.concatenate([acc[0][:, :DMM], (t + pltpu.roll(t, 64, 1))[:, :64]], axis=1)
                    out[pl.ds(r0, seg), pl.ds(0, DM)] = o[MEM:].astype(bf16)
                    state[0] = o[:MEM].astype(bf16).astype(f32)
                yield cst

    ATT_COST = 17408
    per_head = S // seg // H
    assert per_head * H * seg == S and (128 - 3 * L) * (len(GROUPS) - 1) == L

    start(cp_bq + xb_copy(0) + xb_copy(1) + cp_bk + cp_bv + cp_av + cp_a + cp_last)
    ot[...] = jnp.zeros_like(ot)
    wait(cp_bq)
    deinterleave(rawq, wbq, lambda h, e: (h, 0, 128 * e), DM)
    n_t = S // 256 // QN

    def xb_body(m, _):
        _merge((transpose_x(xtb, xb, m), 1))
        return 0
    wait(xb_copy(0))
    lax.fori_loop(0, n_t, xb_body, 0)

    nq, n_kv, n_a = H * QN, DC // CH, DM // CH
    n0 = nq - n_kv - n_a

    def q_body(u, _):
        _merge((b_qproj(u), 1))
        return 0
    lax.fori_loop(0, n0, q_body, 0)
    wait(xb_copy(1))
    lax.fori_loop(n_t, QN * n_t, xb_body, 0)
    wait(cp_bk)

    def q2_body(t, _):
        pl.when(t == n_kv // 2)(lambda: wait(cp_bv))
        w, t2 = t // (n_kv // 2), t % (n_kv // 2)
        de = _chain(*[_deinterleave_chunk(rawkv.at[w], wbkv, lambda h, e: (w * H + h, 0, 128 * e), 2 * t2 + i)
                      for i in range(2)])
        _merge((de, 32 * SL2), (b_qproj(n0 + t), 4096 // QN))
        return 0
    lax.fori_loop(0, n_kv, q2_body, 0)
    wait(cp_av)

    def q3_body(t, _):
        _merge((b_qproj(nq - n_a + t), 4096 // QN),
               (_deinterleave_chunk(raw2, rawq, lambda h, e: (e, h * (DM // 2), 0), t), 16 * SL2))
        return 0
    lax.fori_loop(0, n_a, q3_body, 0)
    wait(cp_a)

    def absorb_body(j, _):
        t = jnp.minimum(j, n_a - 1)
        de = _chain(*[_deinterleave_chunk(raw, wa, lambda h, e, l=l: (h // 2, 0, (h % 2) * 2 * DH + l + 128 * e), t)
                      for raw, l in ((raw0, 0), (raw1, DH))])
        _merge((transpose_x(xta, xa, j), 1), (de, 32 * SL1), (a_absorb(j), 8))
        return 0
    lax.fori_loop(0, H // 2, absorb_body, 0)
    wait(cp_last)

    nb = S // TQ
    a_cost = sum(c_ for _, c_ in ASCHED) * ALEAD

    def head_body(h, mem):
        def kv_body(t, mem):
            state = [mem]
            _merge((a_steps(h * per_head + t, 1, state), a_cost),
                   (_chain(*[b_kvblock(h, t * (nb // 2) + m) for m in range(nb // 2)]), nb // 2 * 2048))
            return state[0]
        state = [lax.fori_loop(0, 2, kv_body, mem)]
        fill = {nb: (b_outproj_acc(h, QORDER[:OSPLIT]), OSPLIT * DM),
                nb + 1: (b_outproj_acc(h, QORDER[OSPLIT:-1]), (nb - 1 - OSPLIT) * DM)}
        _merge((a_steps(h * per_head + 2, per_head - 2, state), (per_head - 2) * a_cost),
               (b_attn(h, fill), ATT_COST + (nb - 1) * DM))
        pl.when(h > 0)(lambda: out_copy_a(h - 1).wait())
        out_copy_a(h).start()
        return state[0]
    lax.fori_loop(0, H, head_body, mem0[...].astype(f32))

    _merge((emit_blocks(QORDER[:-1]), 3 * (nb - 1)), (b_outproj_last(QORDER[-1]), 3 * H))
    wait([out_copy(m) for m in range(S // TQ)] + [out_copy_a(H - 1)])


@functools.partial(jax.jit, static_argnames=("A_seg_len",))
def pallas_concat_heads__memory_aug_recurrent_mem_tr__compressed_kv_cla__prompt_kernel(
    A_x, A_mem0, A_Wq, A_Wk, A_Wv, A_Wo, A_seg_len,
    B_x, B_c_kv, B_w_q, B_w_uk, B_w_uv, B_w_o,
):
    args = (
        A_x.reshape(S, DM).T, A_mem0.reshape(MEM, DM),
        A_Wq.reshape(DM * H, DH), A_Wk.reshape(DM * H, DH), A_Wv.reshape(DM * H, DH),
        A_Wo.transpose(0, 2, 1).reshape(H * DM, DH),
        B_x.reshape(S, DM).T, B_c_kv.reshape(S, DC),
        B_w_q.reshape(DM * H, DH), B_w_uk.reshape(DC * H, DH), B_w_uv.reshape(DC * H, DH),
        B_w_o.transpose(0, 2, 1).reshape(H * DM, DH),
    )
    scratch = [
        pltpu.VMEM((DM, S), bf16),
        pltpu.VMEM((DM, S), bf16),
        pltpu.VMEM((S // 2, DM), u32),
        pltpu.VMEM((S // 2, DM), u32),
        pltpu.VMEM((MEM, DM), bf16),
        pltpu.VMEM((H * DM, DH), bf16),
        pltpu.VMEM((S, DC), bf16),
        pltpu.VMEM((H * DM, DH), bf16),
        pltpu.VMEM((2, DM * 8, 128), u32),
        pltpu.VMEM((2, 2, DC * 8, 128), u32),
        pltpu.VMEM((2, DM * 8, 128), u32),
        pltpu.VMEM((2, DM * 8, 128), u32),
        pltpu.VMEM((2, DM * 8, 128), u32),
        pltpu.VMEM((H // 2, DM // 2, 4 * DH), u32),
        pltpu.VMEM((H // 2, DM // 2, 2 * DMM + 128), u32),
        pltpu.VMEM((H, DM // 2, DH), u32),
        pltpu.VMEM((2 * H, DC // 2, DH), u32),
        pltpu.VMEM((H, S // 2, DH), u32),
        pltpu.VMEM((S // 2, 2 * DH), u32),
        pltpu.VMEM((DM, S), f32),
        pltpu.VMEM((S, 2 * DM), bf16),
        pltpu.SemaphoreType.DMA((20 + S // TQ,)),
    ]
    res = pl.pallas_call(
        functools.partial(_kernel, seg=int(A_seg_len)),
        in_specs=[pl.BlockSpec(memory_space=pl.ANY)] * len(args),
        out_specs=pl.BlockSpec(memory_space=pl.ANY),
        out_shape=jax.ShapeDtypeStruct((S, 2 * DM), bf16),
        scratch_shapes=scratch,
        compiler_params=pltpu.CompilerParams(vmem_limit_bytes=120 << 20),
    )(*args)
    return res.reshape(1, S, 2 * DM)
```

```python
import functools

import jax
import jax.numpy as jnp
import numpy as np
from jax import lax
import jax.experimental.pallas as pl
import jax.experimental.pallas.tpu as pltpu

S = 2048
DM = 448
H = 16
DH = 256
DC = 1024
MEM = 8
TQ = 256
HB = 128
QORDER = (1, 2, 3, 7, 6, 5, 4, 0)
SL1 = 2.1
SL2 = 1.4
OSPLIT = 3
RG = 32
DMM = 384
GROUPS = ((1, 2, 3), (4, 5, 6), (7, 8, 9), (10, 11, 12), (13, 14, 15), (0,))
ASCHED = (("p0", 320), ("p1 s5", 340), ("p2 s0", 380), ("p3 f5", 320), ("p4 s1 f0", 380), ("p5 s2", 380),
          ("p6 f1", 320), ("p7 s3 f2", 380), ("z0 s4", 340), ("z1 f3", 280), ("z2 f4 m0", 320), ("z3", 280),
          ("z4 m1", 320), ("z5 m2", 320), ("z6", 280), ("z7 m3", 320), ("", 200), ("m4", 300))
ALEAD = 1.1
QN = 2
CH = 64
RPAD = 16
NEG = -1000000000.0
SCALE = DH ** -0.5

_NN = (((1,), (0,)), ((), ()))
_NT = (((1,), (1,)), ((), ()))
bf16, f32, u32 = jnp.bfloat16, jnp.float32, jnp.uint32


def _dot(a, b, dims=_NN):
    return lax.dot_general(a, b, dims, preferred_element_type=f32)


def _pack(x):
    return pltpu.bitcast(x.astype(bf16), u32)


def _unpack(x):
    return pltpu.bitcast(x, bf16)


def _deinterleave_chunk(raw, dst, place, t):
    r0 = t * (CH // 2)
    s0 = t * (CH * 8)
    if not isinstance(t, int):
        r0, s0 = pl.multiple_of(r0, CH // 2), pl.multiple_of(s0, CH * 8)
    for half in range(2):
        src = raw.at[half, pl.ds(s0, CH * 8 + RPAD), :]
        for j in range(8):
            xe = src[pl.ds(j, CH // 2, stride=16), :]
            xo = src[pl.ds(8 + j, CH // 2, stride=16), :]
            vals = ((xe & np.uint32(0xFFFF)) | (xo << 16), (xe >> 16) | (xo & np.uint32(0xFFFF0000)))
            for e in range(2):
                i, r, l = place(2 * j + e, half)
                dst[i, pl.ds(r + r0, CH // 2), pl.ds(l, 128)] = vals[e]
            yield 1


def _chain(*gens):
    for g in gens:
        yield from g


def _zip(main, total, side, count):
    done, n = 0.0, 0
    for cst in main:
        done += cst
        while n < count and n < done / total * count:
            next(side)
            n += 1
        yield cst
    for _ in side:
        pass


def _merge(*streams):
    gens = [g for g, _ in streams]
    totals = [float(t) for _, t in streams]
    done = [0.0] * len(gens)
    live = list(range(len(gens)))
    while live:
        i = min(live, key=lambda n: done[n] / totals[n])
        try:
            done[i] += next(gens[i])
        except StopIteration:
            live.remove(i)


def _kernel(xa_hbm, mem_hbm, aq_hbm, ak_hbm, av_hbm, ao_hbm,
            xb_hbm, c_hbm, bq_hbm, bk_hbm, bv_hbm, bo_hbm,
            o_hbm,
            xta, xtb, xa, xb, mem0, wao, c, wbo, rawq, rawkv, raw0, raw1, raw2,
            wa, wz, wbq, wbkv, qc, kv, ot, out, sems, *, seg):
    L = MEM + seg

    def raw_copies(hbm, raw, s0):
        u = hbm.bitcast(u32)
        return [pltpu.make_async_copy(u.at[:, pl.ds(128 * i, 128)], raw.at[i, pl.ds(0, u.shape[0]), :],
                                      sems.at[s0 + i]) for i in range(2)]

    half = S // QN

    def xb_copy(i):
        cols = pl.ds(i * half, half)
        return [pltpu.make_async_copy(xb_hbm.at[:, cols], xtb.at[:, cols], sems.at[i])]

    cp_bq = raw_copies(bq_hbm, rawq, 2)
    cp_bk = raw_copies(bk_hbm, rawkv.at[0], 4)
    cp_bv = raw_copies(bv_hbm, rawkv.at[1], 6)
    cp_av = raw_copies(av_hbm, raw2, 8)
    cp_a = ([pltpu.make_async_copy(ao_hbm, wao, sems.at[10]),
             pltpu.make_async_copy(xa_hbm, xta, sems.at[11])]
            + raw_copies(aq_hbm, raw0, 12) + raw_copies(ak_hbm, raw1, 14))
    cp_last = [pltpu.make_async_copy(mem_hbm, mem0, sems.at[16]),
               pltpu.make_async_copy(c_hbm, c, sems.at[17]),
               pltpu.make_async_copy(bo_hbm, wbo, sems.at[18])]

    def start(cps):
        for cp in cps:
            cp.start()

    def wait(cps):
        for cp in cps:
            cp.wait()

    def transpose_x(xt, xs, m):
        r = pl.multiple_of(m * 128, 128)
        xs[pl.ds(r, 128), :] = pltpu.bitcast(xt[:, pl.ds(pl.multiple_of(2 * r, 256), 256)].T, u32)
        yield 1

    def deinterleave(raw, dst, place, rows):
        def body(t, _):
            _merge((_deinterleave_chunk(raw, dst, place, t), 1))
            return 0
        lax.fori_loop(0, rows // CH, body, 0)

    def b_qproj(u):
        h, m0 = u % H, (u // H) * (S // QN // 2)
        w = _unpack(wbq[h])
        for m in range(S // QN // 256):
            rows = pl.ds(pl.multiple_of(m0 + m * 128, 128), 128)
            qc[h, rows, :] = _pack(_dot(_unpack(xb[rows, :]), w) * SCALE)
            yield 512

    def b_kvblock(h, m):
        r = m * 128
        if not isinstance(m, int):
            r = pl.multiple_of(r, 128)
        for l0 in (0, DH):
            acc = None
            for k0 in range(0, DC, 512):
                d = _dot(c[pl.ds(2 * r, 256), pl.ds(k0, 512)],
                         _unpack(wbkv[(l0 // DH) * H + h, pl.ds(k0 // 2, 256), :]))
                acc = d if acc is None else acc + d
                if k0 + 512 == DC:
                    kv[pl.ds(r, 128), pl.ds(l0, DH)] = _pack(acc)
                yield 512

    def b_attn(h, fill):
        row = lax.broadcasted_iota(jnp.int32, (HB, HB), 0)
        col = lax.broadcasted_iota(jnp.int32, (HB, HB), 1)
        tri = col <= row
        conv = lambda r0, nr, l0: _unpack(kv[pl.ds(r0 // 2, nr // 2), pl.ds(l0, DH)])

        def blocks(i):
            return [(j * TQ, TQ) for j in range(i)] + [(i * TQ, HB)]

        def scores(i, st):
            q = _unpack(qc[h, pl.ds(i * TQ // 2, TQ // 2), :])
            st["s"] = []
            for k0, nk in blocks(i):
                st["s"].append(_dot(q, conv(k0, nk, 0), _NT))
                yield nk
            st["sb"] = _dot(q[HB:], conv(i * TQ + HB, HB, 0), _NT)
            yield HB // 2

        def softmax(i, st):
            st["p"], st["pb"], st["l"] = [], [], []
            for r in range(0, TQ, RG):
                parts = [x[r:r + RG] for x in st["s"]]
                if r < HB:
                    parts[-1] = jnp.where(tri[r:r + RG], parts[-1], NEG)
                else:
                    parts.append(jnp.where(tri[r - HB:r - HB + RG], st["sb"][r - HB:r - HB + RG], NEG))
                s = jnp.concatenate(parts, axis=1)
                p = jnp.exp(s - jnp.max(s, axis=1, keepdims=True))
                st["l"].append(jnp.sum(p, axis=1, keepdims=True))
                p = p.astype(bf16)
                n = i * TQ + HB
                st["p"].append(p[:, :n])
                if r >= HB:
                    st["pb"].append(p[:, n:])
                yield 0

        def values(i, st):
            o = None
            for k0, nk in blocks(i):
                d = _dot(jnp.concatenate([x[:, k0:k0 + nk] for x in st["p"]], axis=0), conv(k0, nk, DH))
                o = d if o is None else o + d
                yield nk
            ob = _dot(jnp.concatenate(st["pb"], axis=0), conv(i * TQ + HB, HB, DH))
            o = jnp.concatenate([o[:HB], o[HB:] + ob], axis=0) / jnp.concatenate(st["l"], axis=0)
            qc[h, pl.ds(i * TQ // 2, TQ // 2), :] = _pack(o)
            yield HB // 2

        cost = lambda i: i * TQ + HB + HB // 2
        sts = [{} for _ in QORDER]
        for t in range(len(QORDER) + 2):
            mxu, tot = [], 0
            if t in fill:
                mxu.append(fill[t][0])
                tot += fill[t][1]
            if t >= 2:
                mxu.append(values(QORDER[t - 2], sts[t - 2]))
                tot += cost(QORDER[t - 2])
            if t < len(QORDER):
                mxu.append(scores(QORDER[t], sts[t]))
                tot += cost(QORDER[t])
            if 1 <= t <= len(QORDER):
                yield from _zip(_chain(*mxu), tot, softmax(QORDER[t - 1], sts[t - 1]), TQ // RG)
            else:
                yield from _chain(*mxu)

    def out_copy(m):
        rows, lanes = pl.ds(m * TQ, TQ), pl.ds(DMM, 2 * DM - DMM)
        return pltpu.make_async_copy(out.at[rows, lanes], o_hbm.at[rows, lanes], sems.at[19 + m])

    def out_copy_a(h):
        n = S // H
        rows, lanes = pl.ds(pl.multiple_of(h * n, n), n), pl.ds(0, DMM)
        return pltpu.make_async_copy(out.at[rows, lanes], o_hbm.at[rows, lanes], sems.at[19 + S // TQ])

    def b_outproj_acc(h, blocks):
        for m in blocks:
            ctx = _unpack(qc[h, pl.ds(m * TQ // 2, TQ // 2), :])
            w = wbo[pl.ds(pl.multiple_of(h * DM, DM), DM), :]
            ot[:, pl.ds(m * TQ, TQ)] += _dot(w, ctx, _NT)
            yield DM

    def emit_block(m, acc):
        out[pl.ds(m * TQ, TQ), pl.ds(DM, DM)] = acc.astype(bf16).T
        out_copy(m).start()

    def b_outproj_last(m):
        acc = None
        for h in range(H):
            ctx = _unpack(qc[h, pl.ds(m * TQ // 2, TQ // 2), :])
            d = _dot(wbo[pl.ds(h * DM, DM), :], ctx, _NT)
            acc = d if acc is None else acc + d
            yield 2
        emit_block(m, acc)

    def emit_blocks(blocks):
        for m in blocks:
            emit_block(m, ot[:, pl.ds(m * TQ, TQ)])
            yield 1

    def a_absorb(j):
        lane = lax.broadcasted_iota(jnp.int32, (DM, 128), 1)
        tails = []
        for e in range(2):
            wrows = pl.ds(pl.multiple_of((2 * j + e) * (DM // 2), 32), DM // 2)
            wv = _unpack(jnp.concatenate([rawq[0, wrows, :], rawq[1, wrows, :]], axis=1))
            r0 = pl.multiple_of((2 * j + e) * DM, 64)
            rt = pl.multiple_of(r0 + DMM - 64 * e, 64)
            wo = jnp.concatenate([wao[pl.ds(r0, DMM), :], wao[pl.ds(rt, 128), :]], axis=0)
            d = _dot(wv, wo, _NT)
            wz[j, :, pl.ds(e * DMM, DMM)] = _pack(d[:, :DMM])
            tails.append(d[:, DMM:])
            yield 4
        wz[j, :, pl.ds(2 * DMM, 128)] = _pack(jnp.where(lane < 64, tails[0], tails[1]))

    def a_steps(s0, nsteps, state):
        row = lax.broadcasted_iota(jnp.int32, (L, 128), 0)
        col = lax.broadcasted_iota(jnp.int32, (L, 128), 1)
        key = col - jnp.where(col >= 2 * L, 2 * L, jnp.where(col >= L, L, 0))
        mask = (row < MEM) | (row >= key)
        spare = 128 - 3 * L
        seg_of = [(col >= g * L) & (col < (g + 1) * L) for g in range(3)]

        def pick(xs):
            r = xs[-1]
            for g in range(len(xs) - 2, -1, -1):
                r = jnp.where(col < (g + 1) * L, xs[g], r)
            return r

        def stack(xs):
            pad = 128 - sum(x.shape[0] for x in xs)
            if pad:
                xs = xs + [jnp.zeros((pad, xs[0].shape[1]), f32)]
            return jnp.concatenate(xs, axis=0).astype(bf16)

        for ds in range(nsteps):
            r0, p0 = (s0 + ds) * seg, (s0 + ds) * (seg // 2)
            r0, p0 = pl.multiple_of(r0, seg), pl.multiple_of(p0, seg // 2)
            hx = jnp.concatenate([state[0], _unpack(xa[pl.ds(p0, seg // 2), :]).astype(f32)], axis=0)
            qs, ks, zs, ss, ps = {}, {}, {}, {}, {}
            acc = [None]

            def project(j):
                qk = _dot(hx, _unpack(wa[j]))
                for e in range(2):
                    qs[2 * j + e] = qk[:, 2 * e * DH:(2 * e + 1) * DH]
                    ks[2 * j + e] = qk[:, (2 * e + 1) * DH:(2 * e + 2) * DH]

            def project_z(j):
                z = _dot(hx, _unpack(wz[j]))
                for e in range(2):
                    tail = jnp.where((col < 64) if e == 0 else (col >= 64), z[:, 2 * DMM:], 0.0)
                    zs[2 * j + e] = jnp.concatenate([z[:, e * DMM:(e + 1) * DMM], tail], axis=1)

            def score(g):
                hs = GROUPS[g]
                r = _dot(jnp.concatenate([qs[h] for h in hs], axis=0), stack([ks[h] for h in hs]), _NT)
                ss[g] = pick([r[n * L:(n + 1) * L] for n in range(len(hs))])

            def soft(g):
                n = len(GROUPS[g])
                s = jnp.where(mask, ss[g] * SCALE, NEG)
                m = pick([jnp.max(jnp.where(seg_of[i], s, -jnp.inf), axis=1, keepdims=True) for i in range(n)])
                p = jnp.where(col < n * L, jnp.exp(s - m), 0.0)
                l = pick([jnp.sum(jnp.where(seg_of[i], p, 0.0), axis=1, keepdims=True) for i in range(n)])
                ps[g] = p / l

            def mix(g):
                last = len(GROUPS) - 1
                p = jnp.where(col < 3 * L, ps[g], pltpu.roll(ps[last], 3 * L - spare * g, 1))
                extra = zs[GROUPS[last][0]][spare * g:spare * (g + 1)]
                d = _dot(p, stack([zs[h] for h in GROUPS[g]] + [extra]))
                acc[0] = d if acc[0] is None else acc[0] + d

            ops = {"p": project, "z": project_z, "s": score, "f": soft, "m": mix}
            for stage, cst in ASCHED:
                for op in stage.split():
                    ops[op[0]](int(op[1]))
                if stage is ASCHED[-1][0]:
                    t = acc[0][:, DMM:]
                    o = jnp.concatenate([acc[0][:, :DMM], (t + pltpu.roll(t, 64, 1))[:, :64]], axis=1)
                    out[pl.ds(r0, seg), pl.ds(0, DM)] = o[MEM:].astype(bf16)
                    state[0] = o[:MEM].astype(bf16).astype(f32)
                yield cst

    ATT_COST = 17408
    per_head = S // seg // H
    assert per_head * H * seg == S and (128 - 3 * L) * (len(GROUPS) - 1) == L

    start(cp_bq + xb_copy(0) + xb_copy(1) + cp_bk + cp_bv + cp_av + cp_a + cp_last)
    ot[...] = jnp.zeros_like(ot)
    wait(cp_bq)
    deinterleave(rawq, wbq, lambda h, e: (h, 0, 128 * e), DM)
    n_t = S // 256 // QN

    def xb_body(m, _):
        _merge((transpose_x(xtb, xb, m), 1))
        return 0
    wait(xb_copy(0))
    lax.fori_loop(0, n_t, xb_body, 0)

    nq, n_kv, n_a = H * QN, DC // CH, DM // CH
    n0 = nq - n_kv - n_a

    def q_body(u, _):
        _merge((b_qproj(u), 1))
        return 0
    lax.fori_loop(0, n0, q_body, 0)
    wait(xb_copy(1))
    lax.fori_loop(n_t, QN * n_t, xb_body, 0)
    wait(cp_bk)

    def q2_body(t, _):
        pl.when(t == n_kv // 2)(lambda: wait(cp_bv))
        w, t2 = t // (n_kv // 2), t % (n_kv // 2)
        de = _chain(*[_deinterleave_chunk(rawkv.at[w], wbkv, lambda h, e: (w * H + h, 0, 128 * e), 2 * t2 + i)
                      for i in range(2)])
        _merge((de, 32 * SL2), (b_qproj(n0 + t), 4096 // QN))
        return 0
    lax.fori_loop(0, n_kv, q2_body, 0)
    wait(cp_av)

    def q3_body(t, _):
        _merge((b_qproj(nq - n_a + t), 4096 // QN),
               (_deinterleave_chunk(raw2, rawq, lambda h, e: (e, h * (DM // 2), 0), t), 16 * SL2))
        return 0
    lax.fori_loop(0, n_a, q3_body, 0)
    wait(cp_a)

    def absorb_body(j, _):
        t = jnp.minimum(j, n_a - 1)
        de = _chain(*[_deinterleave_chunk(raw, wa, lambda h, e, l=l: (h // 2, 0, (h % 2) * 2 * DH + l + 128 * e), t)
                      for raw, l in ((raw0, 0), (raw1, DH))])
        _merge((transpose_x(xta, xa, j), 1), (de, 32 * SL1), (a_absorb(j), 8))
        return 0
    lax.fori_loop(0, H // 2, absorb_body, 0)
    wait(cp_last)

    nb = S // TQ
    a_cost = sum(c_ for _, c_ in ASCHED) * ALEAD

    def head_body(h, mem):
        def kv_body(t, mem):
            state = [mem]
            _merge((a_steps(h * per_head + t, 1, state), a_cost),
                   (_chain(*[b_kvblock(h, t * (nb // 2) + m) for m in range(nb // 2)]), nb // 2 * 2048))
            return state[0]
        state = [lax.fori_loop(0, 2, kv_body, mem)]
        fill = {nb: (b_outproj_acc(h, QORDER[:OSPLIT]), OSPLIT * DM),
                nb + 1: (b_outproj_acc(h, QORDER[OSPLIT:-1]), (nb - 1 - OSPLIT) * DM)}
        _merge((a_steps(h * per_head + 2, per_head - 2, state), (per_head - 2) * a_cost),
               (b_attn(h, fill), ATT_COST + (nb - 1) * DM))
        pl.when(h > 0)(lambda: out_copy_a(h - 1).wait())
        out_copy_a(h).start()
        return state[0]
    lax.fori_loop(0, H, head_body, mem0[...].astype(f32))

    _merge((emit_blocks(QORDER[:-1]), 3 * (nb - 1)), (b_outproj_last(QORDER[-1]), 3 * H))
    wait([out_copy(m) for m in range(S // TQ)] + [out_copy_a(H - 1)])


@functools.partial(jax.jit, static_argnames=("A_seg_len",))
def pallas_concat_heads__memory_aug_recurrent_mem_tr__compressed_kv_cla__prompt_kernel(
    A_x, A_mem0, A_Wq, A_Wk, A_Wv, A_Wo, A_seg_len,
    B_x, B_c_kv, B_w_q, B_w_uk, B_w_uv, B_w_o,
):
    args = (
        A_x.reshape(S, DM).T, A_mem0.reshape(MEM, DM),
        A_Wq.reshape(DM * H, DH), A_Wk.reshape(DM * H, DH), A_Wv.reshape(DM * H, DH),
        A_Wo.transpose(0, 2, 1).reshape(H * DM, DH),
        B_x.reshape(S, DM).T, B_c_kv.reshape(S, DC),
        B_w_q.reshape(DM * H, DH), B_w_uk.reshape(DC * H, DH), B_w_uv.reshape(DC * H, DH),
        B_w_o.transpose(0, 2, 1).reshape(H * DM, DH),
    )
    scratch = [
        pltpu.VMEM((DM, S), bf16),
        pltpu.VMEM((DM, S), bf16),
        pltpu.VMEM((S // 2, DM), u32),
        pltpu.VMEM((S // 2, DM), u32),
        pltpu.VMEM((MEM, DM), bf16),
        pltpu.VMEM((H * DM, DH), bf16),
        pltpu.VMEM((S, DC), bf16),
        pltpu.VMEM((H * DM, DH), bf16),
        pltpu.VMEM((2, DM * 8 + RPAD, 128), u32),
        pltpu.VMEM((2, 2, DC * 8 + RPAD, 128), u32),
        pltpu.VMEM((2, DM * 8 + RPAD, 128), u32),
        pltpu.VMEM((2, DM * 8 + RPAD, 128), u32),
        pltpu.VMEM((2, DM * 8 + RPAD, 128), u32),
        pltpu.VMEM((H // 2, DM // 2, 4 * DH), u32),
        pltpu.VMEM((H // 2, DM // 2, 2 * DMM + 128), u32),
        pltpu.VMEM((H, DM // 2, DH), u32),
        pltpu.VMEM((2 * H, DC // 2, DH), u32),
        pltpu.VMEM((H, S // 2, DH), u32),
        pltpu.VMEM((S // 2, 2 * DH), u32),
        pltpu.VMEM((DM, S), f32),
        pltpu.VMEM((S, 2 * DM), bf16),
        pltpu.SemaphoreType.DMA((20 + S // TQ,)),
    ]
    res = pl.pallas_call(
        functools.partial(_kernel, seg=int(A_seg_len)),
        in_specs=[pl.BlockSpec(memory_space=pl.ANY)] * len(args),
        out_specs=pl.BlockSpec(memory_space=pl.ANY),
        out_shape=jax.ShapeDtypeStruct((S, 2 * DM), bf16),
        scratch_shapes=scratch,
        compiler_params=pltpu.CompilerParams(vmem_limit_bytes=120 << 20),
    )(*args)
    return res.reshape(1, S, 2 * DM)
```
